```python
import os as _os
_os.environ.setdefault("JAX_PLATFORMS", "cpu")
import jax
import jax.numpy as jnp

def _softmax(x, axis=-1):
    return jax.nn.softmax(x, axis=axis)
def _gelu(x):
    return jax.nn.gelu(x, approximate=True)
def _silu(x):
    return jax.nn.silu(x)
def _sigmoid(x):
    return jax.nn.sigmoid(x)
def _layernorm(x, axis=-1, eps=1e-5):
    m = jnp.mean(x, axis=axis, keepdims=True)
    v = jnp.var(x, axis=axis, keepdims=True)
    return (x - m) / jnp.sqrt(v + eps)
def _scatter_add(tgt, idx, src, axis=0):
    return tgt.at[idx].add(src)
def _segment_sum(src, seg, n):
    return jax.ops.segment_sum(src, seg, n)
class _Rng:
    def __init__(self, key):
        self._k = key
    def _next(self):
        self._k, sub = jax.random.split(self._k)
        return sub
    def normal(self, shape):
        return jax.random.normal(self._next(), shape, dtype=jnp.bfloat16)
    def randint(self, lo, hi, shape):
        return jax.random.randint(self._next(), shape, lo, hi, dtype=jnp.int32)
    def uniform(self, shape, lo=0.0, hi=1.0):
        return jax.random.uniform(self._next(), shape, jnp.bfloat16, lo, hi)
    def permutation(self, n):
        return jax.random.permutation(self._next(), n)


kernel_name = 'standalone__batchnorm__sampling'

def setup_inputs():
    _rng = _Rng(jax.random.key(int.from_bytes(__import__("os").urandom(4), "little")))
    _w = (lambda a: (lambda t: t.astype(jnp.bfloat16) if jnp.issubdtype(t.dtype, jnp.floating) else t)(jnp.asarray(a)))
    B, S, C = 1024, 8, 640
    K = 3
    return {
        "x": _w((lambda *s: _rng.normal(s) * 0.05)(B, S, C)),
        "w": _w((lambda *s: _rng.normal(s) * 0.05)(K, C, C) * (1.0 / (K * C) ** 0.5)),
        "mean": _w((lambda *s: _rng.normal(s) * 0.05)(C) * 0.1),
        "var": _w(jnp.abs((lambda *s: _rng.normal(s) * 0.05)(C)) + 0.5),
        "g": _w((lambda *s: _rng.normal(s) * 0.05)(C) + 1.0),
        "b": _w((lambda *s: _rng.normal(s) * 0.05)(C) * 0.1),
    }

def reference(x, w, mean, var, g, b):
    K = 3
    P = K // 2
    S = x.shape[1]
    xp = jnp.pad(x, ((0, 0), (P, P), (0, 0)))
    y = sum(jnp.einsum('bsc,cd->bsd', xp[:, k:k + S, :], w[k]) for k in range(K))
    inv_std = 1.0 / jnp.sqrt(var + 1e-5)
    y = (y - mean) * (g * inv_std) + b
    return _silu(y)
```

```python
import functools
import jax
import jax.numpy as jnp
import jax.experimental.pallas as pl
import jax.experimental.pallas.tpu as pltpu


def _kernel(x_ref, w_ref, mean_ref, var_ref, g_ref, b_ref, o_ref, *, C):
    x = x_ref[...]
    tm = x.shape[0]
    p0 = jnp.dot(x, w_ref[0], preferred_element_type=jnp.float32)
    p1 = jnp.dot(x, w_ref[1], preferred_element_type=jnp.float32)
    p2 = jnp.dot(x, w_ref[2], preferred_element_type=jnp.float32)
    s = jax.lax.broadcasted_iota(jnp.int32, (tm, C), 0) % 8
    p0s = jnp.where(s == 0, 0.0, pltpu.roll(p0, 1, 0))
    p2s = jnp.where(s == 7, 0.0, pltpu.roll(p2, tm - 1, 0))
    y = p0s + p1 + p2s
    mean = mean_ref[...].astype(jnp.float32)
    var = var_ref[...].astype(jnp.float32)
    g = g_ref[...].astype(jnp.float32)
    b = b_ref[...].astype(jnp.float32)
    scale = g * jax.lax.rsqrt(var + 1e-5)
    z = (y - mean) * scale + b
    o_ref[...] = (z * jax.nn.sigmoid(z)).astype(o_ref.dtype)


@jax.jit
def pallas_standalone__batchnorm__sampling_kernel(x, w, mean, var, g, b):
    B, S, C = x.shape
    M = B * S
    TM = 512
    x2 = x.reshape(M, C)
    vec = lambda a: a.reshape(1, C)
    vspec = pl.BlockSpec((1, C), lambda i: (0, 0))
    out = pl.pallas_call(
        functools.partial(_kernel, C=C),
        grid=(M // TM,),
        in_specs=[
            pl.BlockSpec((TM, C), lambda i: (i, 0)),
            pl.BlockSpec((3, C, C), lambda i: (0, 0, 0)),
            vspec, vspec, vspec, vspec,
        ],
        out_specs=pl.BlockSpec((TM, C), lambda i: (i, 0)),
        out_shape=jax.ShapeDtypeStruct((M, C), x.dtype),
        compiler_params=pltpu.CompilerParams(
            dimension_semantics=("arbitrary",),
            vmem_limit_bytes=64 * 1024 * 1024,
        ),
    )(x2, w, vec(mean), vec(var), vec(g), vec(b))
    return out.reshape(B, S, C)
```

```python
import functools
import jax
import jax.numpy as jnp
import numpy as np
import jax.experimental.pallas as pl
import jax.experimental.pallas.tpu as pltpu

def consts(a):
    al = a * a; be = 1.0 / al; kap = al + be
    c1 = (a + 1/a) / 2; s1 = (a - 1/a) / 2
    return dict(a=a, al=al, be=be, kap=kap, c1=c1, s1=s1)

def in_transform(x, a):
    k = consts(a); kap = k['kap']; r = k['s1'] / k['c1']
    x0, x1, x2, x3, x4, x5, x6, x7 = x
    def half(p0, p2, p4, p6):
        s06 = p0 + p6; s24 = p2 + p4
        d60 = p6 - p0; d42 = p4 - p2
        E1 = s06 + s24
        Em1 = d42 - d60
        S = (kap - 1) * s06 + s24
        D = (r * (kap + 1)) * d60 + r * d42
        return E1, Em1, S + D, S - D
    E1, ar, Ep, Em = half(x0, x2, x4, x6)
    O1, ai, Op, Om = half(x1, x3, x5, x7)
    Em = a * Em
    Op = a * Op
    return [x0, x7, ar + ai,
            Ep + Op, Ep - Op, Em + Om, Em - Om,
            E1 + O1, E1 - O1, ar, ai]

def weight_coefs(a):
    k = consts(a); al, be, kap, c1 = k['al'], k['be'], k['kap'], k['c1']
    b = 1 / a
    th_a = 1 / (2 * al * (al * al - 1) * (al - be))
    th_b = 1 / (2 * be * (be * be - 1) * (be - al))
    fa = th_a * (a**3 * c1)
    fb = al * th_b * (c1 / a**4)
    k1 = 1 / (4 * (2 - kap))
    kc = 1 / (2 * (2 + kap))
    G = [
        [1, 0, 0], [0, 0, 1], [0, 1, 0],
        [fa, fa * a, fa * al], [fa, -fa * a, fa * al],
        [fb, fb * b, fb * be], [fb, -fb * b, fb * be],
        [k1, k1, k1], [k1, -k1, k1],
        [kc, kc, -kc], [kc, -kc, -kc],
    ]
    return np.array(G, float), kc

def out_transform(m, a, sc, ksc, csc, sh, sh2):
    k = consts(a); al, be, kap = k['al'], k['be'], k['kap']
    m0, mi, mk, mpa, mma, mpb, mmb, mp1, mm1, k2, k3 = m
    Sa = mpa + mma; Da = mpa - mma
    Sb = mpb + mmb; Db = mpb - mmb
    S1 = mp1 + mm1; D1 = mp1 - mm1
    k1 = csc * mk
    nRe = k1 - k2
    Im = k1 + k3
    e0 = sc * m0
    ke0 = ksc * m0 - sh
    d0 = S1 + nRe
    d1 = S1 - nRe + sh
    e2 = d1 - e0
    c1 = Sa + be * Sb
    nc0 = be * Sa + Sb
    z2 = d0 - ke0 + nc0
    z4 = d1 - kap * d0 - c1
    z6 = (d0 + sh2) - kap * e2 - nc0
    z8 = e2 + c1
    f0 = sc * mi
    kf0 = ksc * mi - sh
    g0 = D1 + Im + sh
    g1 = D1 - Im
    f2 = g0 - f0
    c1p = a * Da + (a**-3) * Db
    nc0p = (1 / a) * (Da + Db)
    z1 = f2 + nc0p
    z3 = (g1 + sh2) - kap * f2 - c1p
    z5 = g0 - kap * g1 - nc0p
    z7 = g1 - kf0 + c1p
    return [z1, z2, z3, z4, z5, z6, z7, z8]


F32 = jnp.float32
BF16 = jnp.bfloat16
U32 = jnp.uint32
NR = 11


def _kernel(x_hbm, w_hbm, mean_ref, var_ref, g_ref, b_ref, o_hbm,
            x_vm, o_vm, w_vm, u_ref, p_ref, pv0, pv1, pv2, pv3, va_ref, vb_ref, m_ref, sem,
            *, B, C, TAIL, HEADV, PROF, A_PT):
    CH = 128
    NT = C // 128
    RW = 4 * NT
    NC = B // CH
    KB = C // 16
    G, kc = weight_coefs(A_PT)
    kap = consts(A_PT)['kap']
    xh = x_hbm.bitcast(U32)
    oh = o_hbm.bitcast(U32)
    wh = w_hbm.bitcast(U32)
    hi_mask = jnp.uint32(0xFFFF0000)
    sign = jnp.uint32(0x80000000)

    def rows(b0, nb):
        if isinstance(b0, int):
            return pl.ds(b0 * RW, nb * RW)
        return pl.ds(pl.multiple_of(b0 * RW, 8), nb * RW)

    def x_copy(b0, nb, s):
        return pltpu.make_async_copy(xh.at[rows(b0, nb), :], x_vm.at[rows(b0, nb), :], sem.at[s])
    def o_copy(b0, nb, s):
        return pltpu.make_async_copy(o_vm.at[rows(b0, nb), :], oh.at[rows(b0, nb), :], sem.at[24 + s])
    def w_copy(n):
        return pltpu.make_async_copy(wh.at[:, :, pl.ds(n * 128, 128)], w_vm.at[n], sem.at[12 + n])

    def itok(src):
        if src is None:
            return jnp.uint32(16), hi_mask
        tb = pltpu.bitcast(src, U32)
        msk = (tb | hi_mask) & hi_mask
        return (msk >> 12) & jnp.uint32(16), msk

    def unpack(wd, tk):
        return pltpu.bitcast(wd << tk[0], F32), pltpu.bitcast(wd & tk[1], F32)

    def pack(a, b):
        return pltpu.pack_elementwise([a, b], packed_dtype=BF16)

    def in_piece(xc, rg, ct, dst):
        def f(src):
            tk = itok(src)
            Vh = []
            for h in range(2):
                xs = []
                for j in range(4):
                    wd = xc[pl.ds((rg * 16 + 8 * h) * RW + ct * 4 + j, 8, stride=RW), :]
                    xs.extend(unpack(wd, tk))
                Vh.append(in_transform(xs, A_PT))
            for r in range(NR):
                dst[r, rg * 8:(rg + 1) * 8, ct * 128:(ct + 1) * 128] = pack(Vh[0][r], Vh[1][r])
        return f

    def out_piece(oc, k, n):
        def f(src):
            cols = slice(n * 128, (n + 1) * 128)
            m = [m_ref[n, r, pl.ds((k // 2) * 16 + (k % 2), 8, stride=2), :] for r in range(NR)]
            sc, ksc, csc, sh, sh2 = [p_ref[i, :, cols] for i in range(5)]
            if src is not None:
                tb = pltpu.bitcast(src, U32)
                tok = pltpu.bitcast((tb | sign) & sign, F32)
                for r in (0, 1, 2, 3, 5, 7):
                    m[r] = m[r] + tok
            hs = out_transform(m, A_PT, sc, ksc, csc, sh, sh2)
            ys = [h + h * jnp.tanh(h) for h in hs]
            for j in range(4):
                oc[pl.ds(k * 8 * RW + n * 4 + j, 8, stride=RW), :] = pack(ys[2 * j], ys[2 * j + 1])
        return f

    def u_piece(n, kbs, groups):
        def f(src):
            tk = itok(src)
            cols = slice(n * 128, (n + 1) * 128)
            for kb in kbs:
                rs = slice(kb * 8, (kb + 1) * 8)
                h0 = unpack(w_vm[n, 2, rs, :], tk)
                h1 = unpack(w_vm[n, 1, rs, :], tk)
                h2 = unpack(w_vm[n, 0, rs, :], tk)
                for gi, base in (('a', 0), ('b', 2), ('c', 4), ('d', 6)):
                    if gi not in groups:
                        continue
                    if gi in 'ab':
                        pi = 5 if gi == 'a' else 8
                        k0 = p_ref[pi, :, cols]; k1 = p_ref[pi + 1, :, cols]; k2 = p_ref[pi + 2, :, cols]
                        e = [k0 * h0[h] + k2 * h2[h] for h in range(2)]
                    elif gi == 'c':
                        k1 = p_ref[11, :, cols]
                        e = [k1 * (h0[h] + h2[h]) for h in range(2)]
                    else:
                        k1 = p_ref[2, :, cols]
                        e = [k1 * (h0[h] - h2[h]) for h in range(2)]
                    o = [k1 * h1[h] for h in range(2)]
                    u_ref[n, base, rs, :] = pack(e[0] + o[0], e[1] + o[1])
                    u_ref[n, base + 1, rs, :] = pack(e[0] - o[0], e[1] - o[1])
        return f

    def run_pass(v, lo, M, n, items, pre=None, rr_range=None):
        rl = list(range(NR)) if rr_range is None else list(rr_range)
        ni = len(items); done = 0
        for ix, r in enumerate(rl):
            if pre is not None and r in pre:
                for f in pre[r]:
                    f(None)
            lhs = pltpu.bitcast(v[r, lo // 2:(lo + M) // 2, :], BF16)
            ru = w_vm[n, (2, 0, 1)[r]] if r < 3 else u_ref[n, r - 3]
            res = jnp.dot(lhs, pltpu.bitcast(ru, BF16), preferred_element_type=F32)
            m_ref[n, r, lo:lo + M, :] = res
            tgt = ((ix + 1) * ni) // len(rl)
            cnt = tgt - done
            for q in range(cnt):
                rr = ((q * (M // 8)) // cnt) * 8
                items[done](res[rr:rr + 8, :])
                done += 1

    def merge(*lists):
        tagged = []
        for l in lists:
            for i, it in enumerate(l):
                tagged.append(((i + 0.5) / len(l), it))
        tagged.sort(key=lambda t: t[0])
        return [t[1] for t in tagged]

    def outs(oc, lo, M, n):
        return [out_piece(oc, k, n) for k in range(lo // 8, (lo + M) // 8)]

    def ins(xc, lo, M, dst):
        return [in_piece(xc, rg, ct, dst) for rg in range(lo // 16, (lo + M) // 16) for ct in range(NT)]

    def us(n, groups='abcd', per=2):
        return [u_piece(n, list(range(k, k + per)), groups) for k in range(0, KB, per)]

    def split(l, k):
        return [l[(i * len(l)) // k:((i + 1) * len(l)) // k] for i in range(k)]

    def xview(b0): return x_vm.at[rows(b0, CH), :]
    def oview(b0): return o_vm.at[rows(b0, CH), :]

    def W(cp, name):
        if PROF:
            with jax.named_scope(name):
                cp.wait()
        else:
            cp.wait()
    nop = lambda s: None

    H = 64
    xc = lambda k: x_copy(k * CH, CH, k + 2)
    xhf = lambda h: x_copy(h * H, H, h)
    oc_ = lambda k: o_copy(k * CH, CH, k)
    pv_ref = [pv0, pv1, pv2, pv3]
    pcs = [pltpu.make_async_copy(r, pv_ref[i], sem.at[18 + i]) for i, r in enumerate((mean_ref, var_ref, g_ref, b_ref))]
    xhf(0).start()
    for cp in pcs: cp.start()
    xhf(1).start()
    for n in range(NT): w_copy(n).start()
    xhf(2).start(); xhf(3).start()
    for k in range(2, NC): xc(k).start()

    x0 = xview(0); o0 = oview(0); x1 = xview(CH); o1 = oview(CH)
    W(xhf(0), "wx0")
    for i, cp in enumerate(pcs): W(cp, "wp%d" % i)
    mean = pv_ref[0][...].astype(F32).reshape(1, C)
    var = pv_ref[1][...].astype(F32).reshape(1, C)
    g = pv_ref[2][...].astype(F32).reshape(1, C)
    b = pv_ref[3][...].astype(F32).reshape(1, C)
    sc = 0.5 * g * jax.lax.rsqrt(var + 1e-5)
    sh = 0.5 * b - mean * sc
    vals = [sc, kap * sc, kc * sc, sh, (1 + kap) * sh]
    vals += [float(G[3, i]) * sc for i in range(3)] + [float(G[5, i]) * sc for i in range(3)] + [float(G[7, 0]) * sc]
    for i, v in enumerate(vals):
        p_ref[i] = jnp.broadcast_to(v, (8, C))

    jit = lambda n: {3: us(n, 'a'), 5: us(n, 'b'), 7: us(n, 'c'), 9: us(n, 'd')}
    O = lambda n: outs(o0, 0, CH, n)
    for f in ins(x0, 0, H, va_ref): f(None)
    W(xhf(1), "wx1")
    for f in ins(x0, H, H, va_ref): f(None)
    if HEADV == 2:
        W(w_copy(0), "ww0")
        run_pass(va_ref, 0, CH, 0, [], pre=jit(0))
        W(w_copy(1), "ww1")
        run_pass(va_ref, 0, CH, 1, [], pre=jit(1))
        W(w_copy(2), "ww2")
        W(w_copy(3), "ww3")
        run_pass(va_ref, 0, CH, 2, [nop] * 20 + us(3), pre=jit(2))
        W(w_copy(4), "ww4")
        W(xhf(2), "wx2")
        run_pass(va_ref, 0, CH, 3, merge(us(4), ins(x1, 0, H, vb_ref)))
        W(xhf(3), "wx3")
        run_pass(va_ref, 0, CH, 4, merge(O(0), ins(x1, H, H, vb_ref)))
        run_pass(vb_ref, 0, CH, 0, O(1) + O(2))
        run_pass(vb_ref, 0, CH, 1, O(3) + O(4) + outs(o1, 0, CH, 0))
        oc_(0).start()

    def body(i, carry):
        c = 2 * i + 1
        W(xc(c + 1), "wxa")
        W(xc(c + 2), "wxb")
        oa = oview(c * CH); ob = oview((c + 1) * CH); oc = oview((c + 2) * CH)
        il = split(ins(xview((c + 1) * CH), 0, CH, va_ref), 3)
        for n in range(2, NT):
            run_pass(vb_ref, 0, CH, n, merge(outs(oa, 0, CH, n - 1), il[n - 2]))
        il = split(ins(xview((c + 2) * CH), 0, CH, vb_ref), NT)
        for n in range(NT):
            ol = outs(oa, 0, CH, NT - 1) if n == 0 else outs(ob, 0, CH, n - 1)
            run_pass(va_ref, 0, CH, n, merge(ol, il[n]))
            if n == 0:
                oc_(c).start()
        run_pass(vb_ref, 0, CH, 0, outs(ob, 0, CH, NT - 1))
        oc_(c + 1).start()
        run_pass(vb_ref, 0, CH, 1, outs(oc, 0, CH, 0))
        return carry
    jax.lax.fori_loop(0, (NC - 2) // 2, body, 0)

    c = NC - 1
    oc = oview(c * CH)
    pend = outs(oc, 0, CH, 1)
    lo = 0
    fin = []
    for ti, M in enumerate(TAIL):
        for n in range(2, NT):
            run_pass(vb_ref, lo, M, n, pend)
            pend = outs(oc, lo, M, n)
            if n == 2 and ti > 0:
                cp = o_copy(c * CH + lo - TAIL[ti - 1], TAIL[ti - 1], c + ti - 1)
                cp.start(); fin.append(cp)
        lo += M
    for f in pend: f(None)
    cp = o_copy(c * CH + lo - TAIL[-1], TAIL[-1], c + len(TAIL) - 1)
    cp.start(); fin.append(cp)
    for k in range(NC - 1):
        W(oc_(k), "wo")
    for cp in fin:
        W(cp, "wof")


def _make(TAIL=(64, 64), HEADV=2, PROF=False, A_PT=1.9):
    @jax.jit
    def f(x, w, mean, var, g, b):
        B, S, C = x.shape
        NT = C // 128
        CH = 128
        z = x.reshape(B, S, NT, 128).transpose(0, 2, 1, 3).reshape(B * S * NT, 128)
        anyspec = pl.BlockSpec(memory_space=pl.ANY)
        scratch = [
            pltpu.VMEM((B * 4 * NT, 128), U32),
            pltpu.VMEM((B * 4 * NT, 128), U32),
            pltpu.VMEM((NT, 3, C // 2, 128), U32),
            pltpu.VMEM((NT, NR - 3, C // 2, 128), U32),
            pltpu.VMEM((12, 8, C), F32),
            pltpu.VMEM((C,), BF16), pltpu.VMEM((C,), BF16), pltpu.VMEM((C,), BF16), pltpu.VMEM((C,), BF16),
            pltpu.VMEM((NR, CH // 2, C), U32),
            pltpu.VMEM((NR, CH // 2, C), U32),
            pltpu.VMEM((NT, NR, CH, 128), F32),
            pltpu.SemaphoreType.DMA((40,)),
        ]
        out = pl.pallas_call(
            functools.partial(_kernel, B=B, C=C, TAIL=TAIL, HEADV=HEADV, PROF=PROF, A_PT=A_PT),
            in_specs=[anyspec] * 6,
            out_specs=anyspec,
            out_shape=jax.ShapeDtypeStruct((B * S * NT, 128), x.dtype),
            scratch_shapes=scratch,
            compiler_params=pltpu.CompilerParams(
                vmem_limit_bytes=100 * 1024 * 1024,
            ),
        )(z, w, mean, var, g, b)
        return out.reshape(B, NT, S, 128).transpose(0, 2, 1, 3).reshape(B, S, C)
    return f


@jax.jit
def pallas_standalone__batchnorm__sampling_kernel(x, w, mean, var, g, b):
    return _make()(x, w, mean, var, g, b)
```

```python
import functools

import jax
import jax.numpy as jnp
import jax.experimental.pallas as pl
import jax.experimental.pallas.tpu as pltpu

F32 = jnp.float32
BF16 = jnp.bfloat16
U32 = jnp.uint32

NR = 11
CH = 128
A_PT = 1.9
_AL = A_PT * A_PT
_BE = 1.0 / _AL
_KAP = _AL + _BE
_C1 = (A_PT + 1.0 / A_PT) / 2.0
_S1 = (A_PT - 1.0 / A_PT) / 2.0
_R = _S1 / _C1
_FA = (A_PT ** 3 * _C1) / (2.0 * _AL * (_AL * _AL - 1.0) * (_AL - _BE))
_FB = _AL * (_C1 / A_PT ** 4) / (2.0 * _BE * (_BE * _BE - 1.0) * (_BE - _AL))
_K1 = 1.0 / (4.0 * (2.0 - _KAP))
_KC = 1.0 / (2.0 * (2.0 + _KAP))

HQ = (32, 32, 32, 32)
HD = 5
HX = 4
TAIL = (64, 32, 32)
TQ = 4
FINE = 2
FINE2 = 3


def _in_transform(x):
    x0, x1, x2, x3, x4, x5, x6, x7 = x

    def half(p0, p2, p4, p6):
        s06 = p0 + p6
        s24 = p2 + p4
        d60 = p6 - p0
        d42 = p4 - p2
        s = (_KAP - 1.0) * s06 + s24
        d = (_R * (_KAP + 1.0)) * d60 + _R * d42
        return s06 + s24, d42 - d60, s + d, s - d

    e1, ar, ep, em = half(x0, x2, x4, x6)
    o1, ai, op, om = half(x1, x3, x5, x7)
    em = A_PT * em
    op = A_PT * op
    return [x0, x7, ar + ai,
            ep + op, ep - op, em + om, em - om,
            e1 + o1, e1 - o1, ar, ai]


def _out_transform(m, sc, ksc, csc, sh, sh2):
    m0, mi, mk, mpa, mma, mpb, mmb, mp1, mm1, k2, k3 = m
    sa = mpa + mma
    da = mpa - mma
    sb = mpb + mmb
    db = mpb - mmb
    s1 = mp1 + mm1
    d1_ = mp1 - mm1
    k1 = csc * mk
    nre = k1 - k2
    im = k1 + k3
    e0 = sc * m0
    ke0 = ksc * m0 - sh
    d0 = s1 + nre
    d1 = s1 - nre + sh
    e2 = d1 - e0
    c1 = sa + _BE * sb
    nc0 = _BE * sa + sb
    z2 = d0 - ke0 + nc0
    z4 = d1 - _KAP * d0 - c1
    z6 = (d0 + sh2) - _KAP * e2 - nc0
    z8 = e2 + c1
    f0 = sc * mi
    kf0 = ksc * mi - sh
    g0 = d1_ + im + sh
    g1 = d1_ - im
    f2 = g0 - f0
    c1p = A_PT * da + (A_PT ** -3) * db
    nc0p = (1.0 / A_PT) * (da + db)
    z1 = f2 + nc0p
    z3 = (g1 + sh2) - _KAP * f2 - c1p
    z5 = g0 - _KAP * g1 - nc0p
    z7 = g1 - kf0 + c1p
    return [z1, z2, z3, z4, z5, z6, z7, z8]


def _kernel(x_hbm, w_hbm, mean_hbm, var_hbm, g_hbm, b_hbm, o_hbm,
            x_vm, o_vm, w_vm, u_ref, p_ref, pv0, pv1, pv2, pv3,
            va_ref, vb_ref, m_ref, sem, *, B, C):
    NT = C // 128
    RW = 4 * NT
    NC = B // CH
    NQ = len(HQ)
    xh = x_hbm.bitcast(U32)
    oh = o_hbm.bitcast(U32)
    wh = w_hbm.bitcast(U32)
    hi_mask = jnp.uint32(0xFFFF0000)
    sign = jnp.uint32(0x80000000)

    s_w = {0: 0, 1: NQ + 1, 2: NQ + 2, 3: NQ + 3, 4: NQ + 3}
    s_x1 = NQ + 4
    s_xp = NQ + 5
    s_out = s_xp + (NC - 2) // 2

    def rows(b0, nb):
        if isinstance(b0, int):
            return pl.ds(b0 * RW, nb * RW)
        return pl.ds(pl.multiple_of(b0 * RW, 8), nb * RW)

    def x_copy(b0, nb, s):
        r = rows(b0, nb)
        return pltpu.make_async_copy(xh.at[r, :], x_vm.at[r, :], sem.at[s])

    def o_rows(r):
        return pltpu.make_async_copy(o_vm.at[r, :], oh.at[r, :], sem.at[s_out])

    def w_copy(n):
        return pltpu.make_async_copy(
            wh.at[:, :, pl.ds(n * 128, 128)], w_vm.at[n], sem.at[s_w[n]])

    def starter(cp):
        return lambda: cp.start()

    def waiter(cp):
        return lambda: cp.wait()

    def dup(t):
        return jnp.concatenate([t, t], axis=0)

    def itok(src):
        if src is None:
            return jnp.uint32(16), hi_mask
        msk = (pltpu.bitcast(src, U32) | hi_mask) & hi_mask
        return dup((msk >> 12) & jnp.uint32(16)), dup(msk)

    def unpack(wd, tk):
        return pltpu.bitcast(wd << tk[0], F32), pltpu.bitcast(wd & tk[1], F32)

    def pack(a, b):
        return pltpu.pack_elementwise([a, b], packed_dtype=BF16)

    def in_piece(xc, rg, ct, dst):
        def f(src):
            tk = itok(src)
            xs = []
            for j in range(4):
                wd = xc[pl.ds(rg * 16 * RW + ct * 4 + j, 16, stride=RW), :]
                xs.extend(unpack(wd, tk))
            v = _in_transform(xs)
            for r in range(NR):
                dst[r, rg * 8:(rg + 1) * 8, ct * 128:(ct + 1) * 128] = pack(v[r][0:8], v[r][8:16])
        return f

    def out_piece(oc, k, n):
        saved = []

        def f0(src):
            saved.append(src)

        def f1(src):
            cols = slice(n * 128, (n + 1) * 128)
            m = [jnp.concatenate(
                [m_ref[n, r, pl.ds(k * 16 + h, 8, stride=2), :] for h in range(2)], axis=0)
                for r in range(NR)]
            prm = [dup(p_ref[i, :, cols]) for i in range(5)]
            if src is not None:
                tb = pltpu.bitcast(jnp.concatenate([saved[0], src], axis=0), U32)
                tok = pltpu.bitcast((tb | sign) & sign, F32)
                for r in (0, 1, 2, 3, 5, 7):
                    m[r] = m[r] + tok
            hs = _out_transform(m, *prm)
            ys = [h + h * jnp.tanh(h) for h in hs]
            for j in range(4):
                oc[pl.ds(k * 16 * RW + n * 4 + j, 16, stride=RW), :] = pack(ys[2 * j], ys[2 * j + 1])
        return [f0, f1]

    def u_piece(n, kb):
        def f(src):
            tk = itok(src)
            cols = slice(n * 128, (n + 1) * 128)
            rs = slice(kb * 16, (kb + 1) * 16)
            h0 = unpack(w_vm[n, 2, rs, :], tk)
            h1 = unpack(w_vm[n, 1, rs, :], tk)
            h2 = unpack(w_vm[n, 0, rs, :], tk)
            for gi in range(4):
                if gi < 2:
                    k0, k1, k2 = [dup(p_ref[5 + 3 * gi + i, :, cols]) for i in range(3)]
                    e = [k0 * h0[h] + k2 * h2[h] for h in range(2)]
                elif gi == 2:
                    k1 = dup(p_ref[11, :, cols])
                    e = [k1 * (h0[h] + h2[h]) for h in range(2)]
                else:
                    k1 = dup(p_ref[2, :, cols])
                    e = [k1 * (h0[h] - h2[h]) for h in range(2)]
                o = [k1 * h1[h] for h in range(2)]
                u_ref[n, 2 * gi, rs, :] = pack(e[0] + o[0], e[1] + o[1])
                u_ref[n, 2 * gi + 1, rs, :] = pack(e[0] - o[0], e[1] - o[1])
        return f

    def outs(oc, lo, M, n):
        return [f for k in range(lo // 16, (lo + M) // 16) for f in out_piece(oc, k, n)]

    def ins(xc, lo, M, dst):
        return [in_piece(xc, rg, ct, dst)
                for rg in range(lo // 16, (lo + M) // 16) for ct in range(NT)]

    def us(n):
        return [u_piece(n, k) for k in range(C // 32)]

    def ung(l):
        return [functools.partial(f, None) for f in l]

    def xview(b0):
        return x_vm.at[rows(b0, CH), :]

    def oview(b0):
        return o_vm.at[rows(b0, CH), :]

    def unit(v, lo, M, n, r):
        lhs = pltpu.bitcast(v[r, lo // 2:(lo + M) // 2, :], BF16)
        ru = w_vm[n, (2, 0, 1)[r]] if r < 3 else u_ref[n, r - 3]
        res = jnp.dot(lhs, pltpu.bitcast(ru, BF16), preferred_element_type=F32)
        m_ref[n, r, lo:lo + M, :] = res
        return res

    def emit(passes, ranges, before, barriers=()):
        units = [(v, lo, M, n, r) for (v, lo, M, n) in passes for r in range(NR)]
        per = [[] for _ in units]
        for items, u0, u1 in ranges:
            for i, it in enumerate(items):
                pos = u0 + (i + 0.5) * (u1 - u0) / len(items)
                per[int(pos)].append((pos - int(pos), it))
        bars = sorted(set([0, len(units)] + list(barriers)))
        halves = set()
        for b0, b1 in zip(bars[:-1], bars[1:]):
            ms = [units[k][2] for k in range(b0, b1)]
            n_same = 0
            for mm in reversed(ms):
                if mm != ms[-1]:
                    break
                n_same += 1
            if (ms[-1] >= 64 and n_same >= 4 and n_same % 4 == 2
                    and ((len(ms) - n_same) * NT) % 4 == 0):
                halves.update((b1 - 1, b1 - 2))
        for ix, (v, lo, M, n, r) in enumerate(units):
            for f in before.get(ix, ()):
                f()
            if ix in halves:
                parts = [unit(v, lo, M // 2, n, r), unit(v, lo + M // 2, M // 2, n, r)]
            else:
                parts = [unit(v, lo, M, n, r)]
            pm = M // len(parts)
            for fr, it in sorted(per[ix], key=lambda t: t[0]):
                rr = int(fr * (M // 8)) * 8
                it(parts[rr // pm][rr % pm:rr % pm + 8, :])
        for f in before.get(len(units), ()):
            f()

    qoff = [sum(HQ[:i]) for i in range(NQ)]
    xq = [x_copy(qoff[i], HQ[i], 1 + i) for i in range(NQ)]
    x1c = x_copy(CH, CH, s_x1)

    def xp(i):
        return x_copy((2 * i + 2) * CH, 2 * CH, s_xp + i)

    def oc_(k):
        return o_rows(rows(k * CH, CH))

    pv = [pv0, pv1, pv2, pv3]
    pcs = [pltpu.make_async_copy(r, pv[i], sem.at[0])
           for i, r in enumerate((mean_hbm, var_hbm, g_hbm, b_hbm))]
    for cp in pcs:
        cp.start()
    w_copy(0).start()
    for cp in xq:
        cp.start()
    for n in range(1, NT):
        w_copy(n).start()
    x1c.start()
    for i in range((NC - 2) // 2):
        xp(i).start()

    for cp in pcs:
        cp.wait()
    w_copy(0).wait()
    mean, var, g, b = [r[...].astype(F32).reshape(1, C) for r in pv]
    sc = 0.5 * g * jax.lax.rsqrt(var + 1e-5)
    sh = 0.5 * b - mean * sc
    prm = [sc, _KAP * sc, _KC * sc, sh, (1.0 + _KAP) * sh,
           _FA * sc, (_FA * A_PT) * sc, (_FA * _AL) * sc,
           _FB * sc, (_FB / A_PT) * sc, (_FB * _BE) * sc, _K1 * sc]
    for i, v in enumerate(prm):
        p_ref[i] = jnp.broadcast_to(v, (8, C))

    x0, o0, x1, o1 = xview(0), oview(0), xview(CH), oview(CH)
    for f in us(0):
        f(None)
    xq[0].wait()
    for f in ins(x0, 0, HQ[0], va_ref):
        f(None)
    passes = ([(va_ref, qoff[i], HQ[i], 0) for i in range(NQ)]
              + [(va_ref, 0, CH, n) for n in range(1, NT)]
              + [(vb_ref, 0, CH, 0), (vb_ref, 0, CH, 1)])
    N1 = (NQ - 1) * NR
    E, Q = 2, 1
    b2, b3, b4 = N1 + 2 * NR - HD, N1 + 3 * NR - HD, N1 + 4 * NR - HD + HX
    before = {i * NR: [waiter(xq[i + 1])] + ung(ins(x0, qoff[i + 1], HQ[i + 1], va_ref))
              for i in range(NQ - 1)}
    before[N1] = [waiter(w_copy(1))]
    before[b2] = [waiter(w_copy(2))]
    before[b3] = [waiter(w_copy(3)), waiter(w_copy(4))]
    before[b4] = [waiter(x1c)]
    barriers = list(before)
    before[N1 + 7 * NR] = [starter(oc_(0))]
    ranges = [
        (us(1), N1, N1 + NR + E),
        (us(2), b2, N1 + 2 * NR + E),
        (us(3), b3, N1 + 3 * NR + E),
        (us(4), N1 + 3 * NR + E, b4 - Q),
        (ins(x1, 0, CH, vb_ref), b4, N1 + 5 * NR - 1),
        (outs(o0, 0, CH, 0), N1 + NR + E, b2 - Q),
        (outs(o0, 0, CH, 1), N1 + 2 * NR + E, b3 - Q),
        (outs(o0, 0, CH, 2) + outs(o0, 0, CH, 3) + outs(o0, 0, CH, 4) + outs(o1, 0, CH, 0),
         N1 + 5 * NR - 1, N1 + 7 * NR - Q),
    ]
    emit(passes, ranges, before, barriers)

    def body(i, carry):
        c = 2 * i + 1
        xp(i).wait()
        oa, ob, oc = oview(c * CH), oview((c + 1) * CH), oview((c + 2) * CH)
        passes = ([(vb_ref, 0, CH, n) for n in range(2, NT)]
                  + [(va_ref, 0, CH, n) for n in range(NT)]
                  + [(vb_ref, 0, CH, 0), (vb_ref, 0, CH, 1)])
        ol = ([outs(oa, 0, CH, n) for n in range(1, NT)]
              + [outs(ob, 0, CH, n) for n in range(NT)] + [outs(oc, 0, CH, 0)])
        last = 2 * NT - 1
        ranges = [(ol[k], k * NR, (k + 1) * NR - (1 if k == last else 0)) for k in range(2 * NT)]
        ranges.append((ins(xview((c + 1) * CH), 0, CH, va_ref), 0, (NT - 2) * NR - 1))
        ranges.append((ins(xview((c + 2) * CH), 0, CH, vb_ref), (NT - 2) * NR, (2 * NT - 2) * NR - 1))
        before = {(NT - 1) * NR: [starter(oc_(c))], last * NR: [starter(oc_(c + 1))]}
        emit(passes, ranges, before)
        return carry

    jax.lax.fori_loop(0, (NC - 2) // 2, body, 0)

    c = NC - 1
    oc = oview(c * CH)
    passes, before = [], {}
    ranges = [(outs(oc, 0, CH, 1), 0, NR)]
    lo = 0
    for ti, M in enumerate(TAIL):
        for n in range(2, NT):
            u0 = len(passes) * NR
            passes.append((vb_ref, lo, M, n))
            if n < NT - 1:
                ranges.append((outs(oc, lo, M, n), u0 + NR, u0 + 2 * NR))
            elif ti < len(TAIL) - 1:
                ranges.append((outs(oc, lo, M, n), u0 + NR, u0 + NR + TQ))
                before[u0 + NR + TQ] = [starter(o_rows(rows(c * CH + lo, M)))]
        lo += M
    M = TAIL[-1]
    lo -= M
    base = (c * CH + lo) * RW

    def grp(gq, p0, p1):
        return [starter(o_rows(pl.ds(base + p * 2 * RW + 8 * gq, 8))) for p in range(p0, p1)]

    its, u0, _ = ranges[-1]
    ranges[-1] = (its, u0, u0 + FINE)
    before[u0 + FINE] = grp(1, 0, M // 2)
    its, u0, _ = ranges[-2]
    ranges[-2] = (its, u0, u0 + FINE2)
    before[u0 + FINE2] = grp(0, 0, M // 2) + grp(3, 0, M // 2)
    ol = outs(oc, lo, M, NT - 1)
    fl = []
    for q in range(M // 16):
        fl += ung(ol[2 * q:2 * q + 2]) + grp(2, 8 * q, 8 * q + 8) + grp(4, 8 * q, 8 * q + 8)
    before[len(passes) * NR] = fl
    emit(passes, ranges, before)
    pltpu.make_async_copy(o_vm, oh, sem.at[s_out]).wait()


@jax.jit
def pallas_standalone__batchnorm__sampling_kernel(x, w, mean, var, g, b):
    B, S, C = x.shape
    NT = C // 128
    assert S == 8 and NT == 5 and B % (2 * CH) == 0 and w.shape == (3, C, C)
    z = x.reshape(B, S, NT, 128).transpose(0, 2, 1, 3).reshape(B * S * NT, 128)
    anyspec = pl.BlockSpec(memory_space=pl.ANY)
    scratch = [
        pltpu.VMEM((B * 4 * NT, 128), U32),
        pltpu.VMEM((B * 4 * NT, 128), U32),
        pltpu.VMEM((NT, 3, C // 2, 128), U32),
        pltpu.VMEM((NT, NR - 3, C // 2, 128), U32),
        pltpu.VMEM((12, 8, C), F32),
        pltpu.VMEM((C,), BF16), pltpu.VMEM((C,), BF16),
        pltpu.VMEM((C,), BF16), pltpu.VMEM((C,), BF16),
        pltpu.VMEM((NR, CH // 2, C), U32),
        pltpu.VMEM((NR, CH // 2, C), U32),
        pltpu.VMEM((NT, NR, CH, 128), F32),
        pltpu.SemaphoreType.DMA((len(HQ) + 6 + (B // CH - 2) // 2,)),
    ]
    out = pl.pallas_call(
        functools.partial(_kernel, B=B, C=C),
        in_specs=[anyspec] * 6,
        out_specs=anyspec,
        out_shape=jax.ShapeDtypeStruct((B * S * NT, 128), x.dtype),
        scratch_shapes=scratch,
        compiler_params=pltpu.CompilerParams(vmem_limit_bytes=100 * 1024 * 1024),
    )(z, w, mean, var, g, b)
    return out.reshape(B, NT, S, 128).transpose(0, 2, 1, 3).reshape(B, S, C)
```

```python
import functools

import jax
import jax.numpy as jnp
import jax.experimental.pallas as pl
import jax.experimental.pallas.tpu as pltpu

F32 = jnp.float32
BF16 = jnp.bfloat16
U32 = jnp.uint32

NR = 11
CH = 128
A_PT = 1.9
_AL = A_PT * A_PT
_BE = 1.0 / _AL
_KAP = _AL + _BE
_C1 = (A_PT + 1.0 / A_PT) / 2.0
_S1 = (A_PT - 1.0 / A_PT) / 2.0
_R = _S1 / _C1
_FA = (A_PT ** 3 * _C1) / (2.0 * _AL * (_AL * _AL - 1.0) * (_AL - _BE))
_FB = _AL * (_C1 / A_PT ** 4) / (2.0 * _BE * (_BE * _BE - 1.0) * (_BE - _AL))
_K1 = 1.0 / (4.0 * (2.0 - _KAP))
_KC = 1.0 / (2.0 * (2.0 + _KAP))

HQ = (32, 32, 32, 32)
HD = 5
HX = 4
TAIL = (64, 32, 32)
TQ = 4


def _in_transform(x):
    x0, x1, x2, x3, x4, x5, x6, x7 = x

    def half(p0, p2, p4, p6):
        s06 = p0 + p6
        s24 = p2 + p4
        d60 = p6 - p0
        d42 = p4 - p2
        s = (_KAP - 1.0) * s06 + s24
        d = (_R * (_KAP + 1.0)) * d60 + _R * d42
        return s06 + s24, d42 - d60, s + d, s - d

    e1, ar, ep, em = half(x0, x2, x4, x6)
    o1, ai, op, om = half(x1, x3, x5, x7)
    em = A_PT * em
    op = A_PT * op
    return [x0, x7, ar + ai,
            ep + op, ep - op, em + om, em - om,
            e1 + o1, e1 - o1, ar, ai]


def _out_transform(m, sc, ksc, csc, sh, sh2):
    m0, mi, mk, mpa, mma, mpb, mmb, mp1, mm1, k2, k3 = m
    sa = mpa + mma
    da = mpa - mma
    sb = mpb + mmb
    db = mpb - mmb
    s1 = mp1 + mm1
    d1_ = mp1 - mm1
    k1 = csc * mk
    nre = k1 - k2
    im = k1 + k3
    e0 = sc * m0
    ke0 = ksc * m0 - sh
    d0 = s1 + nre
    d1 = s1 - nre + sh
    e2 = d1 - e0
    c1 = sa + _BE * sb
    nc0 = _BE * sa + sb
    z2 = d0 - ke0 + nc0
    z4 = d1 - _KAP * d0 - c1
    z6 = (d0 + sh2) - _KAP * e2 - nc0
    z8 = e2 + c1
    f0 = sc * mi
    kf0 = ksc * mi - sh
    g0 = d1_ + im + sh
    g1 = d1_ - im
    f2 = g0 - f0
    c1p = A_PT * da + (A_PT ** -3) * db
    nc0p = (1.0 / A_PT) * (da + db)
    z1 = f2 + nc0p
    z3 = (g1 + sh2) - _KAP * f2 - c1p
    z5 = g0 - _KAP * g1 - nc0p
    z7 = g1 - kf0 + c1p
    return [z1, z2, z3, z4, z5, z6, z7, z8]


def _kernel(x_hbm, w_hbm, mean_hbm, var_hbm, g_hbm, b_hbm, o_hbm,
            x_vm, o_vm, w_vm, u_ref, p_ref, pv0, pv1, pv2, pv3,
            va_ref, vb_ref, m_ref, sem, *, B, C):
    NT = C // 128
    RW = 4 * NT
    NC = B // CH
    NQ = len(HQ)
    xh = x_hbm.bitcast(U32)
    oh = o_hbm.bitcast(U32)
    wh = w_hbm.bitcast(U32)
    hi_mask = jnp.uint32(0xFFFF0000)
    sign = jnp.uint32(0x80000000)

    s_w = {0: 0, 1: NQ + 1, 2: NQ + 2, 3: NQ + 3, 4: NQ + 3}
    s_x1 = NQ + 4
    s_xp = NQ + 5
    s_out = s_xp + (NC - 2) // 2

    def rows(b0, nb):
        if isinstance(b0, int):
            return pl.ds(b0 * RW, nb * RW)
        return pl.ds(pl.multiple_of(b0 * RW, 8), nb * RW)

    def x_copy(b0, nb, s):
        r = rows(b0, nb)
        return pltpu.make_async_copy(xh.at[r, :], x_vm.at[r, :], sem.at[s])

    def o_rows(r):
        return pltpu.make_async_copy(o_vm.at[r, :], oh.at[r, :], sem.at[s_out])

    def w_copy(n):
        return pltpu.make_async_copy(
            wh.at[:, :, pl.ds(n * 128, 128)], w_vm.at[n], sem.at[s_w[n]])

    def starter(cp):
        return lambda: cp.start()

    def waiter(cp):
        return lambda: cp.wait()

    def dup(t):
        return jnp.concatenate([t, t], axis=0)

    def itok(src):
        if src is None:
            return jnp.uint32(16), hi_mask
        msk = (pltpu.bitcast(src, U32) | hi_mask) & hi_mask
        return dup((msk >> 12) & jnp.uint32(16)), dup(msk)

    def unpack(wd, tk):
        return pltpu.bitcast(wd << tk[0], F32), pltpu.bitcast(wd & tk[1], F32)

    def pack(a, b):
        return pltpu.pack_elementwise([a, b], packed_dtype=BF16)

    def in_piece(xc, rg, ct, dst):
        def f(src):
            tk = itok(src)
            xs = []
            for j in range(4):
                wd = xc[pl.ds(rg * 16 * RW + ct * 4 + j, 16, stride=RW), :]
                xs.extend(unpack(wd, tk))
            v = _in_transform(xs)
            for r in range(NR):
                dst[r, rg * 8:(rg + 1) * 8, ct * 128:(ct + 1) * 128] = pack(v[r][0:8], v[r][8:16])
        return f

    def out_piece(oc, k, n):
        saved = []

        def f0(src):
            saved.append(src)

        def f1(src):
            cols = slice(n * 128, (n + 1) * 128)
            m = [jnp.concatenate(
                [m_ref[n, r, pl.ds(k * 16 + h, 8, stride=2), :] for h in range(2)], axis=0)
                for r in range(NR)]
            prm = [dup(p_ref[i, :, cols]) for i in range(5)]
            if src is not None:
                tb = pltpu.bitcast(jnp.concatenate([saved[0], src], axis=0), U32)
                tok = pltpu.bitcast((tb | sign) & sign, F32)
                for r in (0, 1, 2, 3, 5, 7):
                    m[r] = m[r] + tok
            hs = _out_transform(m, *prm)
            ys = [h + h * jnp.tanh(h) for h in hs]
            for j in range(4):
                oc[pl.ds(k * 16 * RW + n * 4 + j, 16, stride=RW), :] = pack(ys[2 * j], ys[2 * j + 1])
        return [f0, f1]

    def u_piece(n, kb):
        def f(src):
            tk = itok(src)
            cols = slice(n * 128, (n + 1) * 128)
            rs = slice(kb * 16, (kb + 1) * 16)
            h0 = unpack(w_vm[n, 2, rs, :], tk)
            h1 = unpack(w_vm[n, 1, rs, :], tk)
            h2 = unpack(w_vm[n, 0, rs, :], tk)
            for gi in range(4):
                if gi < 2:
                    k0, k1, k2 = [dup(p_ref[5 + 3 * gi + i, :, cols]) for i in range(3)]
                    e = [k0 * h0[h] + k2 * h2[h] for h in range(2)]
                elif gi == 2:
                    k1 = dup(p_ref[11, :, cols])
                    e = [k1 * (h0[h] + h2[h]) for h in range(2)]
                else:
                    k1 = dup(p_ref[2, :, cols])
                    e = [k1 * (h0[h] - h2[h]) for h in range(2)]
                o = [k1 * h1[h] for h in range(2)]
                u_ref[n, 2 * gi, rs, :] = pack(e[0] + o[0], e[1] + o[1])
                u_ref[n, 2 * gi + 1, rs, :] = pack(e[0] - o[0], e[1] - o[1])
        return f

    def outs(oc, lo, M, n):
        return [f for k in range(lo // 16, (lo + M) // 16) for f in out_piece(oc, k, n)]

    def ins(xc, lo, M, dst):
        return [in_piece(xc, rg, ct, dst)
                for rg in range(lo // 16, (lo + M) // 16) for ct in range(NT)]

    def us(n):
        return [u_piece(n, k) for k in range(C // 32)]

    def ung(l):
        return [functools.partial(f, None) for f in l]

    def xview(b0):
        return x_vm.at[rows(b0, CH), :]

    def oview(b0):
        return o_vm.at[rows(b0, CH), :]

    def unit(v, lo, M, n, r):
        lhs = pltpu.bitcast(v[r, lo // 2:(lo + M) // 2, :], BF16)
        ru = w_vm[n, (2, 0, 1)[r]] if r < 3 else u_ref[n, r - 3]
        res = jnp.dot(lhs, pltpu.bitcast(ru, BF16), preferred_element_type=F32)
        m_ref[n, r, lo:lo + M, :] = res
        return res

    def emit(passes, ranges, before, barriers=()):
        units = [(v, lo, M, n, r) for (v, lo, M, n) in passes for r in range(NR)]
        per = [[] for _ in units]
        for items, u0, u1 in ranges:
            for i, it in enumerate(items):
                pos = u0 + (i + 0.5) * (u1 - u0) / len(items)
                per[int(pos)].append((pos - int(pos), it))
        bars = sorted(set([0, len(units)] + list(barriers)))
        halves = set()
        for b0, b1 in zip(bars[:-1], bars[1:]):
            ms = [units[k][2] for k in range(b0, b1)]
            n_same = 0
            for mm in reversed(ms):
                if mm != ms[-1]:
                    break
                n_same += 1
            if (ms[-1] >= 64 and n_same >= 4 and n_same % 4 == 2
                    and ((len(ms) - n_same) * NT) % 4 == 0):
                halves.update((b1 - 1, b1 - 2))
        for ix, (v, lo, M, n, r) in enumerate(units):
            for f in before.get(ix, ()):
                f()
            if ix in halves:
                parts = [unit(v, lo, M // 2, n, r), unit(v, lo + M // 2, M // 2, n, r)]
            else:
                parts = [unit(v, lo, M, n, r)]
            pm = M // len(parts)
            for fr, it in sorted(per[ix], key=lambda t: t[0]):
                rr = int(fr * (M // 8)) * 8
                it(parts[rr // pm][rr % pm:rr % pm + 8, :])
        for f in before.get(len(units), ()):
            f()

    qoff = [sum(HQ[:i]) for i in range(NQ)]
    xq = [x_copy(qoff[i], HQ[i], 1 + i) for i in range(NQ)]
    x1c = x_copy(CH, CH, s_x1)

    def xp(i):
        return x_copy((2 * i + 2) * CH, 2 * CH, s_xp + i)

    def oc_(k):
        return o_rows(rows(k * CH, CH))

    pv = [pv0, pv1, pv2, pv3]
    pcs = [pltpu.make_async_copy(r, pv[i], sem.at[0])
           for i, r in enumerate((mean_hbm, var_hbm, g_hbm, b_hbm))]
    for cp in pcs:
        cp.start()
    w_copy(0).start()
    for cp in xq:
        cp.start()
    for n in range(1, NT):
        w_copy(n).start()
    x1c.start()
    for i in range((NC - 2) // 2):
        xp(i).start()

    for cp in pcs:
        cp.wait()
    w_copy(0).wait()
    mean, var, g, b = [r[...].astype(F32).reshape(1, C) for r in pv]
    sc = 0.5 * g * jax.lax.rsqrt(var + 1e-5)
    sh = 0.5 * b - mean * sc
    prm = [sc, _KAP * sc, _KC * sc, sh, (1.0 + _KAP) * sh,
           _FA * sc, (_FA * A_PT) * sc, (_FA * _AL) * sc,
           _FB * sc, (_FB / A_PT) * sc, (_FB * _BE) * sc, _K1 * sc]
    for i, v in enumerate(prm):
        p_ref[i] = jnp.broadcast_to(v, (8, C))

    x0, o0, x1, o1 = xview(0), oview(0), xview(CH), oview(CH)
    for f in us(0):
        f(None)
    xq[0].wait()
    for f in ins(x0, 0, HQ[0], va_ref):
        f(None)
    passes = ([(va_ref, qoff[i], HQ[i], 0) for i in range(NQ)]
              + [(va_ref, 0, CH, n) for n in range(1, NT)]
              + [(vb_ref, 0, CH, 0), (vb_ref, 0, CH, 1)])
    N1 = (NQ - 1) * NR
    E, Q = 2, 1
    b2, b3, b4 = N1 + 2 * NR - HD, N1 + 3 * NR - HD, N1 + 4 * NR - HD + HX
    before = {i * NR: [waiter(xq[i + 1])] + ung(ins(x0, qoff[i + 1], HQ[i + 1], va_ref))
              for i in range(NQ - 1)}
    before[N1] = [waiter(w_copy(1))]
    before[b2] = [waiter(w_copy(2))]
    before[b3] = [waiter(w_copy(3)), waiter(w_copy(4))]
    before[b4] = [waiter(x1c)]
    barriers = list(before)
    before[N1 + 7 * NR] = [starter(oc_(0))]
    ranges = [
        (us(1), N1, N1 + NR + E),
        (us(2), b2, N1 + 2 * NR + E),
        (us(3), b3, N1 + 3 * NR + E),
        (us(4), N1 + 3 * NR + E, b4 - Q),
        (ins(x1, 0, CH, vb_ref), b4, N1 + 5 * NR - 1),
        (outs(o0, 0, CH, 0), N1 + NR + E, b2 - Q),
        (outs(o0, 0, CH, 1), N1 + 2 * NR + E, b3 - Q),
        (outs(o0, 0, CH, 2) + outs(o0, 0, CH, 3) + outs(o0, 0, CH, 4) + outs(o1, 0, CH, 0),
         N1 + 5 * NR - 1, N1 + 7 * NR - Q),
    ]
    emit(passes, ranges, before, barriers)

    def body(i, carry):
        c = 2 * i + 1
        xp(i).wait()
        oa, ob, oc = oview(c * CH), oview((c + 1) * CH), oview((c + 2) * CH)
        passes = ([(vb_ref, 0, CH, n) for n in range(2, NT)]
                  + [(va_ref, 0, CH, n) for n in range(NT)]
                  + [(vb_ref, 0, CH, 0), (vb_ref, 0, CH, 1)])
        ol = ([outs(oa, 0, CH, n) for n in range(1, NT)]
              + [outs(ob, 0, CH, n) for n in range(NT)] + [outs(oc, 0, CH, 0)])
        last = 2 * NT - 1
        ranges = [(ol[k], k * NR, (k + 1) * NR - (1 if k == last else 0)) for k in range(2 * NT)]
        ranges.append((ins(xview((c + 1) * CH), 0, CH, va_ref), 0, (NT - 2) * NR - 1))
        ranges.append((ins(xview((c + 2) * CH), 0, CH, vb_ref), (NT - 2) * NR, (2 * NT - 2) * NR - 1))
        before = {(NT - 1) * NR: [starter(oc_(c))], last * NR: [starter(oc_(c + 1))]}
        emit(passes, ranges, before)
        return carry

    jax.lax.fori_loop(0, (NC - 2) // 2, body, 0)

    c = NC - 1
    oc = oview(c * CH)
    passes, before = [], {}
    ranges = [(outs(oc, 0, CH, 1), 0, NR)]
    lo = 0
    for ti, M in enumerate(TAIL):
        for n in range(2, NT):
            u0 = len(passes) * NR
            passes.append((vb_ref, lo, M, n))
            if n < NT - 1:
                ranges.append((outs(oc, lo, M, n), u0 + NR, u0 + 2 * NR))
            elif ti < len(TAIL) - 1:
                ranges.append((outs(oc, lo, M, n), u0 + NR, u0 + NR + TQ))
                before[u0 + NR + TQ] = [starter(o_rows(rows(c * CH + lo, M)))]
        lo += M
    M = TAIL[-1]
    lo -= M
    before[len(passes) * NR] = (ung(outs(oc, lo, M, NT - 1))
                                + [starter(o_rows(rows(c * CH + lo, M)))])
    emit(passes, ranges, before)
    pltpu.make_async_copy(o_vm, oh, sem.at[s_out]).wait()


@jax.jit
def pallas_standalone__batchnorm__sampling_kernel(x, w, mean, var, g, b):
    B, S, C = x.shape
    NT = C // 128
    assert S == 8 and NT == 5 and B % (2 * CH) == 0 and w.shape == (3, C, C)
    z = x.reshape(B, S, NT, 128).transpose(0, 2, 1, 3).reshape(B * S * NT, 128)
    anyspec = pl.BlockSpec(memory_space=pl.ANY)
    scratch = [
        pltpu.VMEM((B * 4 * NT, 128), U32),
        pltpu.VMEM((B * 4 * NT, 128), U32),
        pltpu.VMEM((NT, 3, C // 2, 128), U32),
        pltpu.VMEM((NT, NR - 3, C // 2, 128), U32),
        pltpu.VMEM((12, 8, C), F32),
        pltpu.VMEM((C,), BF16), pltpu.VMEM((C,), BF16),
        pltpu.VMEM((C,), BF16), pltpu.VMEM((C,), BF16),
        pltpu.VMEM((NR, CH // 2, C), U32),
        pltpu.VMEM((NR, CH // 2, C), U32),
        pltpu.VMEM((NT, NR, CH, 128), F32),
        pltpu.SemaphoreType.DMA((len(HQ) + 6 + (B // CH - 2) // 2,)),
    ]
    out = pl.pallas_call(
        functools.partial(_kernel, B=B, C=C),
        in_specs=[anyspec] * 6,
        out_specs=anyspec,
        out_shape=jax.ShapeDtypeStruct((B * S * NT, 128), x.dtype),
        scratch_shapes=scratch,
        compiler_params=pltpu.CompilerParams(vmem_limit_bytes=100 * 1024 * 1024),
    )(z, w, mean, var, g, b)
    return out.reshape(B, NT, S, 128).transpose(0, 2, 1, 3).reshape(B, S, C)
```

```python
import functools

import jax
import jax.numpy as jnp
import jax.experimental.pallas as pl
import jax.experimental.pallas.tpu as pltpu

F32 = jnp.float32
BF16 = jnp.bfloat16
U32 = jnp.uint32

NR = 11
CH = 128
A_PT = 1.9
_AL = A_PT * A_PT
_BE = 1.0 / _AL
_KAP = _AL + _BE
_C1 = (A_PT + 1.0 / A_PT) / 2.0
_S1 = (A_PT - 1.0 / A_PT) / 2.0
_R = _S1 / _C1
_FA = (A_PT ** 3 * _C1) / (2.0 * _AL * (_AL * _AL - 1.0) * (_AL - _BE))
_FB = _AL * (_C1 / A_PT ** 4) / (2.0 * _BE * (_BE * _BE - 1.0) * (_BE - _AL))
_K1 = 1.0 / (4.0 * (2.0 - _KAP))
_KC = 1.0 / (2.0 * (2.0 + _KAP))

HQ = (32, 32, 32, 32)
HD = 5
HX = 4
TAIL = (64, 32, 32)
TQ = 4
FINE = 3


def _in_transform(x):
    x0, x1, x2, x3, x4, x5, x6, x7 = x

    def half(p0, p2, p4, p6):
        s06 = p0 + p6
        s24 = p2 + p4
        d60 = p6 - p0
        d42 = p4 - p2
        s = (_KAP - 1.0) * s06 + s24
        d = (_R * (_KAP + 1.0)) * d60 + _R * d42
        return s06 + s24, d42 - d60, s + d, s - d

    e1, ar, ep, em = half(x0, x2, x4, x6)
    o1, ai, op, om = half(x1, x3, x5, x7)
    em = A_PT * em
    op = A_PT * op
    return [x0, x7, ar + ai,
            ep + op, ep - op, em + om, em - om,
            e1 + o1, e1 - o1, ar, ai]


def _out_transform(m, sc, ksc, csc, sh, sh2):
    m0, mi, mk, mpa, mma, mpb, mmb, mp1, mm1, k2, k3 = m
    sa = mpa + mma
    da = mpa - mma
    sb = mpb + mmb
    db = mpb - mmb
    s1 = mp1 + mm1
    d1_ = mp1 - mm1
    k1 = csc * mk
    nre = k1 - k2
    im = k1 + k3
    e0 = sc * m0
    ke0 = ksc * m0 - sh
    d0 = s1 + nre
    d1 = s1 - nre + sh
    e2 = d1 - e0
    c1 = sa + _BE * sb
    nc0 = _BE * sa + sb
    z2 = d0 - ke0 + nc0
    z4 = d1 - _KAP * d0 - c1
    z6 = (d0 + sh2) - _KAP * e2 - nc0
    z8 = e2 + c1
    f0 = sc * mi
    kf0 = ksc * mi - sh
    g0 = d1_ + im + sh
    g1 = d1_ - im
    f2 = g0 - f0
    c1p = A_PT * da + (A_PT ** -3) * db
    nc0p = (1.0 / A_PT) * (da + db)
    z1 = f2 + nc0p
    z3 = (g1 + sh2) - _KAP * f2 - c1p
    z5 = g0 - _KAP * g1 - nc0p
    z7 = g1 - kf0 + c1p
    return [z1, z2, z3, z4, z5, z6, z7, z8]


def _kernel(x_hbm, w_hbm, mean_hbm, var_hbm, g_hbm, b_hbm, o_hbm,
            x_vm, o_vm, o2_vm, w_vm, u_ref, p_ref, pv0, pv1, pv2, pv3,
            va_ref, vb_ref, m_ref, sem, *, B, C):
    NT = C // 128
    RW = 4 * NT
    NC = B // CH
    NQ = len(HQ)
    xh = x_hbm.bitcast(U32)
    oh = o_hbm.bitcast(U32)
    wh = w_hbm.bitcast(U32)
    hi_mask = jnp.uint32(0xFFFF0000)
    sign = jnp.uint32(0x80000000)

    s_w = {0: 0, 1: NQ + 1, 2: NQ + 2, 3: NQ + 3, 4: NQ + 3}
    s_x1 = NQ + 4
    s_xp = NQ + 5
    s_out = s_xp + (NC - 2) // 2

    def rows(b0, nb):
        if isinstance(b0, int):
            return pl.ds(b0 * RW, nb * RW)
        return pl.ds(pl.multiple_of(b0 * RW, 8), nb * RW)

    def x_copy(b0, nb, s):
        r = rows(b0, nb)
        return pltpu.make_async_copy(xh.at[r, :], x_vm.at[r, :], sem.at[s])

    def o_rows(r):
        return pltpu.make_async_copy(o_vm.at[r, :], oh.at[r, :], sem.at[s_out])

    def w_copy(n):
        return pltpu.make_async_copy(
            wh.at[:, :, pl.ds(n * 128, 128)], w_vm.at[n], sem.at[s_w[n]])

    def starter(cp):
        return lambda: cp.start()

    def waiter(cp):
        return lambda: cp.wait()

    def dup(t):
        return jnp.concatenate([t, t], axis=0)

    def itok(src):
        if src is None:
            return jnp.uint32(16), hi_mask
        msk = (pltpu.bitcast(src, U32) | hi_mask) & hi_mask
        return dup((msk >> 12) & jnp.uint32(16)), dup(msk)

    def unpack(wd, tk):
        return pltpu.bitcast(wd << tk[0], F32), pltpu.bitcast(wd & tk[1], F32)

    def pack(a, b):
        return pltpu.pack_elementwise([a, b], packed_dtype=BF16)

    def in_piece(xc, rg, ct, dst):
        def f(src):
            tk = itok(src)
            xs = []
            for j in range(4):
                wd = xc[pl.ds(rg * 16 * RW + ct * 4 + j, 16, stride=RW), :]
                xs.extend(unpack(wd, tk))
            v = _in_transform(xs)
            for r in range(NR):
                dst[r, rg * 8:(rg + 1) * 8, ct * 128:(ct + 1) * 128] = pack(v[r][0:8], v[r][8:16])
        return f

    def out_piece(oc, k, n, last_chunk):
        k2 = k - (CH - TAIL[-1]) // 16
        stage = last_chunk and k2 >= 0 and n in (0, 3, 4)
        saved = []

        def f0(src):
            saved.append(src)

        def f1(src):
            cols = slice(n * 128, (n + 1) * 128)
            m = [jnp.concatenate(
                [m_ref[n, r, pl.ds(k * 16 + h, 8, stride=2), :] for h in range(2)], axis=0)
                for r in range(NR)]
            prm = [dup(p_ref[i, :, cols]) for i in range(5)]
            if src is not None:
                tb = pltpu.bitcast(jnp.concatenate([saved[0], src], axis=0), U32)
                tok = pltpu.bitcast((tb | sign) & sign, F32)
                for r in (0, 1, 2, 3, 5, 7):
                    m[r] = m[r] + tok
            hs = _out_transform(m, *prm)
            ys = [h + h * jnp.tanh(h) for h in hs]
            for j in range(4):
                pk = pack(ys[2 * j], ys[2 * j + 1])
                if not (stage and n == NT - 1):
                    oc[pl.ds(k * 16 * RW + n * 4 + j, 16, stride=RW), :] = pk
                if stage:
                    o2_vm[pl.ds(k2 * 16 * RW + n * 4 + j, 16, stride=RW), :] = pk
        return [f0, f1]

    def u_piece(n, kb):
        def f(src):
            tk = itok(src)
            cols = slice(n * 128, (n + 1) * 128)
            rs = slice(kb * 16, (kb + 1) * 16)
            h0 = unpack(w_vm[n, 2, rs, :], tk)
            h1 = unpack(w_vm[n, 1, rs, :], tk)
            h2 = unpack(w_vm[n, 0, rs, :], tk)
            for gi in range(4):
                if gi < 2:
                    k0, k1, k2 = [dup(p_ref[5 + 3 * gi + i, :, cols]) for i in range(3)]
                    e = [k0 * h0[h] + k2 * h2[h] for h in range(2)]
                elif gi == 2:
                    k1 = dup(p_ref[11, :, cols])
                    e = [k1 * (h0[h] + h2[h]) for h in range(2)]
                else:
                    k1 = dup(p_ref[2, :, cols])
                    e = [k1 * (h0[h] - h2[h]) for h in range(2)]
                o = [k1 * h1[h] for h in range(2)]
                u_ref[n, 2 * gi, rs, :] = pack(e[0] + o[0], e[1] + o[1])
                u_ref[n, 2 * gi + 1, rs, :] = pack(e[0] - o[0], e[1] - o[1])
        return f

    def outs(oc, lo, M, n, last_chunk=False):
        return [f for k in range(lo // 16, (lo + M) // 16) for f in out_piece(oc, k, n, last_chunk)]

    def ins(xc, lo, M, dst):
        return [in_piece(xc, rg, ct, dst)
                for rg in range(lo // 16, (lo + M) // 16) for ct in range(NT)]

    def us(n):
        return [u_piece(n, k) for k in range(C // 32)]

    def ung(l):
        return [functools.partial(f, None) for f in l]

    def xview(b0):
        return x_vm.at[rows(b0, CH), :]

    def oview(b0):
        return o_vm.at[rows(b0, CH), :]

    def unit(v, lo, M, n, r):
        lhs = pltpu.bitcast(v[r, lo // 2:(lo + M) // 2, :], BF16)
        ru = w_vm[n, (2, 0, 1)[r]] if r < 3 else u_ref[n, r - 3]
        res = jnp.dot(lhs, pltpu.bitcast(ru, BF16), preferred_element_type=F32)
        m_ref[n, r, lo:lo + M, :] = res
        return res

    def emit(passes, ranges, before, barriers=()):
        units = [(v, lo, M, n, r) for (v, lo, M, n) in passes for r in range(NR)]
        per = [[] for _ in units]
        for items, u0, u1 in ranges:
            for i, it in enumerate(items):
                pos = u0 + (i + 0.5) * (u1 - u0) / len(items)
                per[int(pos)].append((pos - int(pos), it))
        bars = sorted(set([0, len(units)] + list(barriers)))
        halves = set()
        for b0, b1 in zip(bars[:-1], bars[1:]):
            ms = [units[k][2] for k in range(b0, b1)]
            n_same = 0
            for mm in reversed(ms):
                if mm != ms[-1]:
                    break
                n_same += 1
            if (ms[-1] >= 64 and n_same >= 4 and n_same % 4 == 2
                    and ((len(ms) - n_same) * NT) % 4 == 0):
                halves.update((b1 - 1, b1 - 2))
        for ix, (v, lo, M, n, r) in enumerate(units):
            for f in before.get(ix, ()):
                f()
            if ix in halves:
                parts = [unit(v, lo, M // 2, n, r), unit(v, lo + M // 2, M // 2, n, r)]
            else:
                parts = [unit(v, lo, M, n, r)]
            pm = M // len(parts)
            for fr, it in sorted(per[ix], key=lambda t: t[0]):
                rr = int(fr * (M // 8)) * 8
                it(parts[rr // pm][rr % pm:rr % pm + 8, :])
        for f in before.get(len(units), ()):
            f()

    qoff = [sum(HQ[:i]) for i in range(NQ)]
    xq = [x_copy(qoff[i], HQ[i], 1 + i) for i in range(NQ)]
    x1c = x_copy(CH, CH, s_x1)

    def xp(i):
        return x_copy((2 * i + 2) * CH, 2 * CH, s_xp + i)

    def oc_(k):
        return o_rows(rows(k * CH, CH))

    pv = [pv0, pv1, pv2, pv3]
    pcs = [pltpu.make_async_copy(r, pv[i], sem.at[0])
           for i, r in enumerate((mean_hbm, var_hbm, g_hbm, b_hbm))]
    for cp in pcs:
        cp.start()
    w_copy(0).start()
    for cp in xq:
        cp.start()
    for n in range(1, NT):
        w_copy(n).start()
    x1c.start()
    for i in range((NC - 2) // 2):
        xp(i).start()

    for cp in pcs:
        cp.wait()
    w_copy(0).wait()
    mean, var, g, b = [r[...].astype(F32).reshape(1, C) for r in pv]
    sc = 0.5 * g * jax.lax.rsqrt(var + 1e-5)
    sh = 0.5 * b - mean * sc
    prm = [sc, _KAP * sc, _KC * sc, sh, (1.0 + _KAP) * sh,
           _FA * sc, (_FA * A_PT) * sc, (_FA * _AL) * sc,
           _FB * sc, (_FB / A_PT) * sc, (_FB * _BE) * sc, _K1 * sc]
    for i, v in enumerate(prm):
        p_ref[i] = jnp.broadcast_to(v, (8, C))

    x0, o0, x1, o1 = xview(0), oview(0), xview(CH), oview(CH)
    for f in us(0):
        f(None)
    xq[0].wait()
    for f in ins(x0, 0, HQ[0], va_ref):
        f(None)
    passes = ([(va_ref, qoff[i], HQ[i], 0) for i in range(NQ)]
              + [(va_ref, 0, CH, n) for n in range(1, NT)]
              + [(vb_ref, 0, CH, 0), (vb_ref, 0, CH, 1)])
    N1 = (NQ - 1) * NR
    E, Q = 2, 1
    b2, b3, b4 = N1 + 2 * NR - HD, N1 + 3 * NR - HD, N1 + 4 * NR - HD + HX
    before = {i * NR: [waiter(xq[i + 1])] + ung(ins(x0, qoff[i + 1], HQ[i + 1], va_ref))
              for i in range(NQ - 1)}
    before[N1] = [waiter(w_copy(1))]
    before[b2] = [waiter(w_copy(2))]
    before[b3] = [waiter(w_copy(3)), waiter(w_copy(4))]
    before[b4] = [waiter(x1c)]
    barriers = list(before)
    before[N1 + 7 * NR] = [starter(oc_(0))]
    ranges = [
        (us(1), N1, N1 + NR + E),
        (us(2), b2, N1 + 2 * NR + E),
        (us(3), b3, N1 + 3 * NR + E),
        (us(4), N1 + 3 * NR + E, b4 - Q),
        (ins(x1, 0, CH, vb_ref), b4, N1 + 5 * NR - 1),
        (outs(o0, 0, CH, 0), N1 + NR + E, b2 - Q),
        (outs(o0, 0, CH, 1), N1 + 2 * NR + E, b3 - Q),
        (outs(o0, 0, CH, 2) + outs(o0, 0, CH, 3) + outs(o0, 0, CH, 4) + outs(o1, 0, CH, 0),
         N1 + 5 * NR - 1, N1 + 7 * NR - Q),
    ]
    emit(passes, ranges, before, barriers)

    def body(i, carry):
        c = 2 * i + 1
        xp(i).wait()
        oa, ob, oc = oview(c * CH), oview((c + 1) * CH), oview((c + 2) * CH)
        passes = ([(vb_ref, 0, CH, n) for n in range(2, NT)]
                  + [(va_ref, 0, CH, n) for n in range(NT)]
                  + [(vb_ref, 0, CH, 0), (vb_ref, 0, CH, 1)])
        ol = ([outs(oa, 0, CH, n) for n in range(1, NT)]
              + [outs(ob, 0, CH, n) for n in range(NT)] + [outs(oc, 0, CH, 0, True)])
        last = 2 * NT - 1
        ranges = [(ol[k], k * NR, (k + 1) * NR - (1 if k == last else 0)) for k in range(2 * NT)]
        ranges.append((ins(xview((c + 1) * CH), 0, CH, va_ref), 0, (NT - 2) * NR - 1))
        ranges.append((ins(xview((c + 2) * CH), 0, CH, vb_ref), (NT - 2) * NR, (2 * NT - 2) * NR - 1))
        before = {(NT - 1) * NR: [starter(oc_(c))], last * NR: [starter(oc_(c + 1))]}
        emit(passes, ranges, before)
        return carry

    jax.lax.fori_loop(0, (NC - 2) // 2, body, 0)

    c = NC - 1
    oc = oview(c * CH)
    passes, before = [], {}
    ranges = [(outs(oc, 0, CH, 1), 0, NR)]
    lo = 0
    for ti, M in enumerate(TAIL):
        for n in range(2, NT):
            u0 = len(passes) * NR
            passes.append((vb_ref, lo, M, n))
            if n < NT - 1:
                ranges.append((outs(oc, lo, M, n, True), u0 + NR, u0 + 2 * NR))
            elif ti < len(TAIL) - 1:
                ranges.append((outs(oc, lo, M, n), u0 + NR, u0 + NR + TQ))
                before[u0 + NR + TQ] = [starter(o_rows(rows(c * CH + lo, M)))]
        lo += M
    M = TAIL[-1]
    lo -= M
    base = (c * CH + lo) * RW
    its, u0, _ = ranges[-1]
    ranges[-1] = (its, u0, u0 + FINE)
    before[u0 + FINE] = [starter(o_rows(pl.ds(base + p * 2 * RW + r0, nr)))
                         for p in range(M // 2) for r0, nr in ((0, 16), (24, 8))]
    ol = outs(oc, lo, M, NT - 1, True)
    fl = []
    for q in range(M // 16):
        fl += ung(ol[2 * q:2 * q + 2])
        for p in range(8 * q, 8 * q + 8):
            for r0 in (16, 32):
                fl.append(starter(pltpu.make_async_copy(
                    o2_vm.at[pl.ds(p * 2 * RW + r0, 8), :],
                    oh.at[pl.ds(base + p * 2 * RW + r0, 8), :], sem.at[s_out])))
    before[len(passes) * NR] = fl
    emit(passes, ranges, before)
    pltpu.make_async_copy(oh, oh, sem.at[s_out]).wait()


@jax.jit
def pallas_standalone__batchnorm__sampling_kernel(x, w, mean, var, g, b):
    B, S, C = x.shape
    NT = C // 128
    assert S == 8 and NT == 5 and B % (2 * CH) == 0 and w.shape == (3, C, C)
    z = x.reshape(B, S, NT, 128).transpose(0, 2, 1, 3).reshape(B * S * NT, 128)
    anyspec = pl.BlockSpec(memory_space=pl.ANY)
    scratch = [
        pltpu.VMEM((B * 4 * NT, 128), U32),
        pltpu.VMEM((B * 4 * NT, 128), U32),
        pltpu.VMEM((TAIL[-1] * 4 * NT, 128), U32),
        pltpu.VMEM((NT, 3, C // 2, 128), U32),
        pltpu.VMEM((NT, NR - 3, C // 2, 128), U32),
        pltpu.VMEM((12, 8, C), F32),
        pltpu.VMEM((C,), BF16), pltpu.VMEM((C,), BF16),
        pltpu.VMEM((C,), BF16), pltpu.VMEM((C,), BF16),
        pltpu.VMEM((NR, CH // 2, C), U32),
        pltpu.VMEM((NR, CH // 2, C), U32),
        pltpu.VMEM((NT, NR, CH, 128), F32),
        pltpu.SemaphoreType.DMA((len(HQ) + 6 + (B // CH - 2) // 2,)),
    ]
    out = pl.pallas_call(
        functools.partial(_kernel, B=B, C=C),
        in_specs=[anyspec] * 6,
        out_specs=anyspec,
        out_shape=jax.ShapeDtypeStruct((B * S * NT, 128), x.dtype),
        scratch_shapes=scratch,
        compiler_params=pltpu.CompilerParams(vmem_limit_bytes=100 * 1024 * 1024),
    )(z, w, mean, var, g, b)
    return out.reshape(B, NT, S, 128).transpose(0, 2, 1, 3).reshape(B, S, C)
```

```python
import functools
import itertools

import jax
import jax.numpy as jnp
import jax.experimental.pallas as pl
import jax.experimental.pallas.tpu as pltpu

F32 = jnp.float32
BF16 = jnp.bfloat16
U32 = jnp.uint32

NR = 11
CH = 128
A_PT = 1.9
_AL = A_PT * A_PT
_BE = 1.0 / _AL
_KAP = _AL + _BE
_C1 = (A_PT + 1.0 / A_PT) / 2.0
_S1 = (A_PT - 1.0 / A_PT) / 2.0
_R = _S1 / _C1
_FA = (A_PT ** 3 * _C1) / (2.0 * _AL * (_AL * _AL - 1.0) * (_AL - _BE))
_FB = _AL * (_C1 / A_PT ** 4) / (2.0 * _BE * (_BE * _BE - 1.0) * (_BE - _AL))
_K1 = 1.0 / (4.0 * (2.0 - _KAP))
_KC = 1.0 / (2.0 * (2.0 + _KAP))

HQ = (32, 32, 32, 32)
HD = 5
HX = 4
TAIL = (64, 32, 32)
TQ = 4
FINE = 3
HE = 2
HE1 = 2
NO = 8
NO1 = 8


def _in_transform(x):
    x0, x1, x2, x3, x4, x5, x6, x7 = x

    def half(p0, p2, p4, p6):
        s06 = p0 + p6
        s24 = p2 + p4
        d60 = p6 - p0
        d42 = p4 - p2
        s = (_KAP - 1.0) * s06 + s24
        d = (_R * (_KAP + 1.0)) * d60 + _R * d42
        return s06 + s24, d42 - d60, s + d, s - d

    e1, ar, ep, em = half(x0, x2, x4, x6)
    o1, ai, op, om = half(x1, x3, x5, x7)
    em = A_PT * em
    op = A_PT * op
    return [x0, x7, ar + ai,
            ep + op, ep - op, em + om, em - om,
            e1 + o1, e1 - o1, ar, ai]


def _out_transform(m, sc, ksc, csc, sh, sh2):
    m0, mi, mk, mpa, mma, mpb, mmb, mp1, mm1, k2, k3 = m
    sa = mpa + mma
    da = mpa - mma
    sb = mpb + mmb
    db = mpb - mmb
    s1 = mp1 + mm1
    d1_ = mp1 - mm1
    k1 = csc * mk
    nre = k1 - k2
    im = k1 + k3
    e0 = sc * m0
    ke0 = ksc * m0 - sh
    d0 = s1 + nre
    d1 = s1 - nre + sh
    e2 = d1 - e0
    c1 = sa + _BE * sb
    nc0 = _BE * sa + sb
    z2 = d0 - ke0 + nc0
    z4 = d1 - _KAP * d0 - c1
    z6 = (d0 + sh2) - _KAP * e2 - nc0
    z8 = e2 + c1
    f0 = sc * mi
    kf0 = ksc * mi - sh
    g0 = d1_ + im + sh
    g1 = d1_ - im
    f2 = g0 - f0
    c1p = A_PT * da + (A_PT ** -3) * db
    nc0p = (1.0 / A_PT) * (da + db)
    z1 = f2 + nc0p
    z3 = (g1 + sh2) - _KAP * f2 - c1p
    z5 = g0 - _KAP * g1 - nc0p
    z7 = g1 - kf0 + c1p
    return [z1, z2, z3, z4, z5, z6, z7, z8]


def _kernel(x_hbm, w_hbm, mean_hbm, var_hbm, g_hbm, b_hbm, o_hbm,
            x_vm, o_vm, o2_vm, w_vm, u_ref, p_ref, pv0, pv1, pv2, pv3,
            va_ref, vb_ref, m_ref, sem, *, B, C):
    NT = C // 128
    RW = 4 * NT
    NC = B // CH
    NQ = len(HQ)
    xh = x_hbm.bitcast(U32)
    oh = o_hbm.bitcast(U32)
    wh = w_hbm.bitcast(U32)
    hi_mask = jnp.uint32(0xFFFF0000)
    sign = jnp.uint32(0x80000000)

    s_w = {0: 0, 1: NQ + 1, 2: NQ + 2, 3: NQ + 3, 4: NQ + 3}
    s_x1 = NQ + 4
    s_xp = NQ + 5
    s_out = s_xp + (NC - 2) // 2

    def rows(b0, nb):
        if isinstance(b0, int):
            return pl.ds(b0 * RW, nb * RW)
        return pl.ds(pl.multiple_of(b0 * RW, 8), nb * RW)

    def x_copy(b0, nb, s):
        r = rows(b0, nb)
        return pltpu.make_async_copy(xh.at[r, :], x_vm.at[r, :], sem.at[s])

    def o_rows(r):
        return pltpu.make_async_copy(o_vm.at[r, :], oh.at[r, :], sem.at[s_out])

    def w_copy(n):
        return pltpu.make_async_copy(
            wh.at[:, :, pl.ds(n * 128, 128)], w_vm.at[n], sem.at[s_w[n]])

    def starter(cp):
        return lambda: cp.start()

    def waiter(cp):
        return lambda: cp.wait()

    def dup(t):
        return jnp.concatenate([t, t], axis=0)

    def itok(src):
        if src is None:
            return jnp.uint32(16), hi_mask
        msk = (pltpu.bitcast(src, U32) | hi_mask) & hi_mask
        return dup((msk >> 12) & jnp.uint32(16)), dup(msk)

    def unpack(wd, tk):
        return pltpu.bitcast(wd << tk[0], F32), pltpu.bitcast(wd & tk[1], F32)

    def pack(a, b):
        return pltpu.pack_elementwise([a, b], packed_dtype=BF16)

    def in_piece(xc, rg, ct, dst):
        def f(src):
            tk = itok(src)
            xs = []
            for j in range(4):
                wd = xc[pl.ds(rg * 16 * RW + ct * 4 + j, 16, stride=RW), :]
                xs.extend(unpack(wd, tk))
            v = _in_transform(xs)
            for r in range(NR):
                dst[r, rg * 8:(rg + 1) * 8, ct * 128:(ct + 1) * 128] = pack(v[r][0:8], v[r][8:16])
        return f

    def out_piece(oc, k, n, last_chunk):
        k2 = k - (CH - TAIL[-1]) // 16
        stage = last_chunk and k2 >= 0 and n in (0, 3, 4)
        saved = []

        def f0(src):
            saved.append(src)

        def f1(src):
            cols = slice(n * 128, (n + 1) * 128)
            m = [jnp.concatenate(
                [m_ref[n, r, pl.ds(k * 16 + h, 8, stride=2), :] for h in range(2)], axis=0)
                for r in range(NR)]
            prm = [dup(p_ref[i, :, cols]) for i in range(5)]
            if src is not None:
                tb = pltpu.bitcast(jnp.concatenate([saved[0], src], axis=0), U32)
                tok = pltpu.bitcast((tb | sign) & sign, F32)
                for r in (0, 1, 2, 3, 5, 7):
                    m[r] = m[r] + tok
            hs = _out_transform(m, *prm)
            ys = [h + h * jnp.tanh(h) for h in hs]
            for j in range(4):
                pk = pack(ys[2 * j], ys[2 * j + 1])
                if not (stage and n == NT - 1):
                    oc[pl.ds(k * 16 * RW + n * 4 + j, 16, stride=RW), :] = pk
                if stage:
                    o2_vm[pl.ds(k2 * 16 * RW + n * 4 + j, 16, stride=RW), :] = pk
        return [f0, f1]

    def u_piece(n, kb):
        def f(src):
            tk = itok(src)
            cols = slice(n * 128, (n + 1) * 128)
            rs = slice(kb * 16, (kb + 1) * 16)
            h0 = unpack(w_vm[n, 2, rs, :], tk)
            h1 = unpack(w_vm[n, 1, rs, :], tk)
            h2 = unpack(w_vm[n, 0, rs, :], tk)
            for gi in range(4):
                if gi < 2:
                    k0, k1, k2 = [dup(p_ref[5 + 3 * gi + i, :, cols]) for i in range(3)]
                    e = [k0 * h0[h] + k2 * h2[h] for h in range(2)]
                elif gi == 2:
                    k1 = dup(p_ref[11, :, cols])
                    e = [k1 * (h0[h] + h2[h]) for h in range(2)]
                else:
                    k1 = dup(p_ref[2, :, cols])
                    e = [k1 * (h0[h] - h2[h]) for h in range(2)]
                o = [k1 * h1[h] for h in range(2)]
                u_ref[n, 2 * gi, rs, :] = pack(e[0] + o[0], e[1] + o[1])
                u_ref[n, 2 * gi + 1, rs, :] = pack(e[0] - o[0], e[1] - o[1])
        return f

    def outs(oc, lo, M, n, last_chunk=False):
        return [f for k in range(lo // 16, (lo + M) // 16) for f in out_piece(oc, k, n, last_chunk)]

    def ins(xc, lo, M, dst):
        return [in_piece(xc, rg, ct, dst)
                for rg in range(lo // 16, (lo + M) // 16) for ct in range(NT)]

    def us(n):
        return [u_piece(n, k) for k in range(C // 32)]

    def ung(l):
        return [functools.partial(f, None) for f in l]

    def xview(b0):
        return x_vm.at[rows(b0, CH), :]

    def oview(b0):
        return o_vm.at[rows(b0, CH), :]

    def unit(v, lo, M, n, r):
        lhs = pltpu.bitcast(v[r, lo // 2:(lo + M) // 2, :], BF16)
        ru = w_vm[n, (2, 0, 1)[r]] if r < 3 else u_ref[n, r - 3]
        res = jnp.dot(lhs, pltpu.bitcast(ru, BF16), preferred_element_type=F32)
        m_ref[n, r, lo:lo + M, :] = res
        return res

    def emit(passes, ranges, before, barriers=()):
        units = [(v, lo, M, n, r) for (v, lo, M, n) in passes for r in range(NR)]
        per = [[] for _ in units]
        for items, u0, u1 in ranges:
            tot = sum(units[k][2] for k in range(u0, u1))
            k, acc = u0, 0
            for i, it in enumerate(items):
                pos = (i + 0.5) * tot / len(items)
                while pos >= acc + units[k][2]:
                    acc += units[k][2]
                    k += 1
                per[k].append(((pos - acc) / units[k][2], it))
        bars = sorted(set([0, len(units)] + list(barriers)))
        nsplit = {}
        for b0, b1 in zip(bars[:-1], bars[1:]):
            cand = list(range(max(b0, b1 - 4), b1))
            best = None
            for combo in itertools.product((1, 2, 4), repeat=len(cand)):
                sp = dict(zip(cand, combo))
                if any(units[k][2] // v < 32 for k, v in sp.items() if v > 1):
                    continue
                load, t = [0] * 4, 0
                for k in range(b0, b1):
                    v = sp.get(k, 1)
                    for _ in range(v * NT):
                        load[t % 4] += units[k][2] // v
                        t += 1
                key = (max(load), sum(combo))
                if best is None or key < best[0]:
                    best = (key, sp)
            nsplit.update(best[1])
        for ix, (v, lo, M, n, r) in enumerate(units):
            for f in before.get(ix, ()):
                f()
            ns = nsplit.get(ix, 1)
            parts = [unit(v, lo + q * (M // ns), M // ns, n, r) for q in range(ns)]
            pm = M // len(parts)
            for fr, it in sorted(per[ix], key=lambda t: t[0]):
                rr = int(fr * (M // 8)) * 8
                it(parts[rr // pm][rr % pm:rr % pm + 8, :])
        for f in before.get(len(units), ()):
            f()

    qoff = [sum(HQ[:i]) for i in range(NQ)]
    xq = [x_copy(qoff[i], HQ[i], 1 + i) for i in range(NQ)]
    x1c = x_copy(CH, CH, s_x1)

    def xp(i):
        return x_copy((2 * i + 2) * CH, 2 * CH, s_xp + i)

    def oc_(k):
        return o_rows(rows(k * CH, CH))

    pv = [pv0, pv1, pv2, pv3]
    pcs = [pltpu.make_async_copy(r, pv[i], sem.at[0])
           for i, r in enumerate((mean_hbm, var_hbm, g_hbm, b_hbm))]
    for cp in pcs:
        cp.start()
    w_copy(0).start()
    for cp in xq:
        cp.start()
    for n in range(1, NT):
        w_copy(n).start()
    x1c.start()
    for i in range((NC - 2) // 2):
        xp(i).start()

    for cp in pcs:
        cp.wait()
    w_copy(0).wait()
    mean, var, g, b = [r[...].astype(F32).reshape(1, C) for r in pv]
    sc = 0.5 * g * jax.lax.rsqrt(var + 1e-5)
    sh = 0.5 * b - mean * sc
    prm = [sc, _KAP * sc, _KC * sc, sh, (1.0 + _KAP) * sh,
           _FA * sc, (_FA * A_PT) * sc, (_FA * _AL) * sc,
           _FB * sc, (_FB / A_PT) * sc, (_FB * _BE) * sc, _K1 * sc]
    for i, v in enumerate(prm):
        p_ref[i] = jnp.broadcast_to(v, (8, C))

    x0, o0, x1, o1 = xview(0), oview(0), xview(CH), oview(CH)
    for f in us(0):
        f(None)
    xq[0].wait()
    for f in ins(x0, 0, HQ[0], va_ref):
        f(None)
    passes = ([(va_ref, qoff[i], HQ[i], 0) for i in range(NQ)]
              + [(va_ref, 0, CH, n) for n in range(1, NT)]
              + [(vb_ref, 0, CH, 0), (vb_ref, 0, CH, 1)])
    N1 = (NQ - 1) * NR
    E, Q = HE, 1
    b2, b3, b4 = N1 + 2 * NR - HD, N1 + 3 * NR - HD, N1 + 4 * NR - HD + HX
    before = {i * NR: [waiter(xq[i + 1])] + ung(ins(x0, qoff[i + 1], HQ[i + 1], va_ref))
              for i in range(NQ - 1)}
    before[N1] = [waiter(w_copy(1))]
    before[b2] = [waiter(w_copy(2))]
    before[b3] = [waiter(w_copy(3)), waiter(w_copy(4))]
    before[b4] = [waiter(x1c)]
    barriers = list(before)
    oo0, oo1 = outs(o0, 0, CH, 0), outs(o0, 0, CH, 1)
    if NO:
        before[b2] += ung(oo0[-NO:])
        oo0 = oo0[:-NO]
    if NO1:
        before[b3] += ung(oo1[-NO1:])
        oo1 = oo1[:-NO1]
    before[N1 + 7 * NR] = [starter(oc_(0))]
    ranges = [
        (us(1), N1, N1 + NR + HE1),
        (us(2), b2, N1 + 2 * NR + E),
        (us(3), b3, N1 + 3 * NR + E),
        (us(4), N1 + 3 * NR + E, b4 - Q),
        (ins(x1, 0, CH, vb_ref), b4, N1 + 5 * NR - 1),
        (oo0, N1 + NR + E, b2 - Q),
        (oo1, N1 + 2 * NR + E, b3 - Q),
        (outs(o0, 0, CH, 2) + outs(o0, 0, CH, 3) + outs(o0, 0, CH, 4) + outs(o1, 0, CH, 0),
         N1 + 5 * NR - 1, N1 + 7 * NR - Q),
    ]
    emit(passes, ranges, before, barriers)

    def body(i, carry):
        c = 2 * i + 1
        xp(i).wait()
        oa, ob, oc = oview(c * CH), oview((c + 1) * CH), oview((c + 2) * CH)
        passes = ([(vb_ref, 0, CH, n) for n in range(2, NT)]
                  + [(va_ref, 0, CH, n) for n in range(NT)]
                  + [(vb_ref, 0, CH, 0), (vb_ref, 0, CH, 1)])
        ol = ([outs(oa, 0, CH, n) for n in range(1, NT)]
              + [outs(ob, 0, CH, n) for n in range(NT)] + [outs(oc, 0, CH, 0, True)])
        last = 2 * NT - 1
        ranges = [(ol[k], k * NR, (k + 1) * NR - (1 if k == last else 0)) for k in range(2 * NT)]
        ranges.append((ins(xview((c + 1) * CH), 0, CH, va_ref), 0, (NT - 2) * NR - 1))
        ranges.append((ins(xview((c + 2) * CH), 0, CH, vb_ref), (NT - 2) * NR, (2 * NT - 2) * NR - 1))
        before = {(NT - 1) * NR: [starter(oc_(c))], last * NR: [starter(oc_(c + 1))]}
        emit(passes, ranges, before)
        return carry

    jax.lax.fori_loop(0, (NC - 2) // 2, body, 0)

    c = NC - 1
    oc = oview(c * CH)
    passes, before = [], {}
    ranges = [(outs(oc, 0, CH, 1), 0, NR)]
    lo = 0
    for ti, M in enumerate(TAIL):
        for n in range(2, NT):
            u0 = len(passes) * NR
            passes.append((vb_ref, lo, M, n))
            if n < NT - 1:
                ranges.append((outs(oc, lo, M, n, True), u0 + NR, u0 + 2 * NR))
            elif ti < len(TAIL) - 1:
                ranges.append((outs(oc, lo, M, n), u0 + NR, u0 + NR + TQ))
                before[u0 + NR + TQ] = [starter(o_rows(rows(c * CH + lo, M)))]
        lo += M
    M = TAIL[-1]
    lo -= M
    base = (c * CH + lo) * RW
    its, u0, _ = ranges[-1]
    ranges[-1] = (its, u0, u0 + FINE)
    before[u0 + FINE] = [starter(o_rows(pl.ds(base + p * 2 * RW + r0, nr)))
                         for p in range(M // 2) for r0, nr in ((0, 16), (24, 8))]
    ol = outs(oc, lo, M, NT - 1, True)
    fl = []
    for q in range(M // 16):
        fl += ung(ol[2 * q:2 * q + 2])
        for p in range(8 * q, 8 * q + 8):
            for r0 in (16, 32):
                fl.append(starter(pltpu.make_async_copy(
                    o2_vm.at[pl.ds(p * 2 * RW + r0, 8), :],
                    oh.at[pl.ds(base + p * 2 * RW + r0, 8), :], sem.at[s_out])))
    before[len(passes) * NR] = fl
    emit(passes, ranges, before)
    pltpu.make_async_copy(oh, oh, sem.at[s_out]).wait()


@jax.jit
def pallas_standalone__batchnorm__sampling_kernel(x, w, mean, var, g, b):
    B, S, C = x.shape
    NT = C // 128
    assert S == 8 and NT == 5 and B % (2 * CH) == 0 and w.shape == (3, C, C)
    z = x.reshape(B, S, NT, 128).transpose(0, 2, 1, 3).reshape(B * S * NT, 128)
    anyspec = pl.BlockSpec(memory_space=pl.ANY)
    scratch = [
        pltpu.VMEM((B * 4 * NT, 128), U32),
        pltpu.VMEM((B * 4 * NT, 128), U32),
        pltpu.VMEM((TAIL[-1] * 4 * NT, 128), U32),
        pltpu.VMEM((NT, 3, C // 2, 128), U32),
        pltpu.VMEM((NT, NR - 3, C // 2, 128), U32),
        pltpu.VMEM((12, 8, C), F32),
        pltpu.VMEM((C,), BF16), pltpu.VMEM((C,), BF16),
        pltpu.VMEM((C,), BF16), pltpu.VMEM((C,), BF16),
        pltpu.VMEM((NR, CH // 2, C), U32),
        pltpu.VMEM((NR, CH // 2, C), U32),
        pltpu.VMEM((NT, NR, CH, 128), F32),
        pltpu.SemaphoreType.DMA((len(HQ) + 6 + (B // CH - 2) // 2,)),
    ]
    out = pl.pallas_call(
        functools.partial(_kernel, B=B, C=C),
        in_specs=[anyspec] * 6,
        out_specs=anyspec,
        out_shape=jax.ShapeDtypeStruct((B * S * NT, 128), x.dtype),
        scratch_shapes=scratch,
        compiler_params=pltpu.CompilerParams(vmem_limit_bytes=100 * 1024 * 1024),
    )(z, w, mean, var, g, b)
    return out.reshape(B, NT, S, 128).transpose(0, 2, 1, 3).reshape(B, S, C)
```

```python
import functools
import itertools

import jax
import jax.numpy as jnp
import jax.experimental.pallas as pl
import jax.experimental.pallas.tpu as pltpu

F32 = jnp.float32
BF16 = jnp.bfloat16
U32 = jnp.uint32

NR = 11
CH = 128
A_PT = 1.9
_AL = A_PT * A_PT
_BE = 1.0 / _AL
_KAP = _AL + _BE
_C1 = (A_PT + 1.0 / A_PT) / 2.0
_S1 = (A_PT - 1.0 / A_PT) / 2.0
_R = _S1 / _C1
_FA = (A_PT ** 3 * _C1) / (2.0 * _AL * (_AL * _AL - 1.0) * (_AL - _BE))
_FB = _AL * (_C1 / A_PT ** 4) / (2.0 * _BE * (_BE * _BE - 1.0) * (_BE - _AL))
_K1 = 1.0 / (4.0 * (2.0 - _KAP))
_KC = 1.0 / (2.0 * (2.0 + _KAP))

HQ = (32, 32, 32, 32)
HD = 5
HX = 4
HE = 2
HE1 = 2
NO = 8
NO1 = 8
TAIL = (64, 32, 32)
TQ = 4
FINE = 3


def _in_transform(x):
    x0, x1, x2, x3, x4, x5, x6, x7 = x

    def half(p0, p2, p4, p6):
        s06 = p0 + p6
        s24 = p2 + p4
        d60 = p6 - p0
        d42 = p4 - p2
        s = (_KAP - 1.0) * s06 + s24
        d = (_R * (_KAP + 1.0)) * d60 + _R * d42
        return s06 + s24, d42 - d60, s + d, s - d

    e1, ar, ep, em = half(x0, x2, x4, x6)
    o1, ai, op, om = half(x1, x3, x5, x7)
    em = A_PT * em
    op = A_PT * op
    return [x0, x7, ar + ai,
            ep + op, ep - op, em + om, em - om,
            e1 + o1, e1 - o1, ar, ai]


def _out_transform(m, sc, ksc, csc, sh, sh2):
    m0, mi, mk, mpa, mma, mpb, mmb, mp1, mm1, k2, k3 = m
    sa = mpa + mma
    da = mpa - mma
    sb = mpb + mmb
    db = mpb - mmb
    s1 = mp1 + mm1
    d1_ = mp1 - mm1
    k1 = csc * mk
    nre = k1 - k2
    im = k1 + k3
    e0 = sc * m0
    ke0 = ksc * m0 - sh
    d0 = s1 + nre
    d1 = s1 - nre + sh
    e2 = d1 - e0
    c1 = sa + _BE * sb
    nc0 = _BE * sa + sb
    z2 = d0 - ke0 + nc0
    z4 = d1 - _KAP * d0 - c1
    z6 = (d0 + sh2) - _KAP * e2 - nc0
    z8 = e2 + c1
    f0 = sc * mi
    kf0 = ksc * mi - sh
    g0 = d1_ + im + sh
    g1 = d1_ - im
    f2 = g0 - f0
    c1p = A_PT * da + (A_PT ** -3) * db
    nc0p = (1.0 / A_PT) * (da + db)
    z1 = f2 + nc0p
    z3 = (g1 + sh2) - _KAP * f2 - c1p
    z5 = g0 - _KAP * g1 - nc0p
    z7 = g1 - kf0 + c1p
    return [z1, z2, z3, z4, z5, z6, z7, z8]


def _kernel(x_hbm, w_hbm, mean_hbm, var_hbm, g_hbm, b_hbm, o_hbm,
            x_vm, o_vm, o2_vm, w_vm, u_ref, p_ref, pv0, pv1, pv2, pv3,
            va_ref, vb_ref, m_ref, sem, *, B, C):
    NT = C // 128
    RW = 4 * NT
    NC = B // CH
    NQ = len(HQ)
    xh = x_hbm.bitcast(U32)
    oh = o_hbm.bitcast(U32)
    hi_mask = jnp.uint32(0xFFFF0000)
    sign = jnp.uint32(0x80000000)

    s_w = {0: 0, 1: NQ + 1, 2: NQ + 2, 3: NQ + 3, 4: NQ + 3}
    s_x1 = NQ + 4
    s_xp = NQ + 5
    s_out = s_xp + (NC - 2) // 2

    def rows(b0, nb):
        if isinstance(b0, int):
            return pl.ds(b0 * RW, nb * RW)
        return pl.ds(pl.multiple_of(b0 * RW, 8), nb * RW)

    def x_copy(b0, nb, s):
        r = rows(b0, nb)
        return pltpu.make_async_copy(xh.at[r, :], x_vm.at[r, :], sem.at[s])

    def o_rows(r):
        return pltpu.make_async_copy(o_vm.at[r, :], oh.at[r, :], sem.at[s_out])

    def w_copy(n):
        return pltpu.make_async_copy(
            w_hbm.at[:, :, pl.ds(n * 128, 128)], w_vm.at[n], sem.at[s_w[n]])

    def starter(cp):
        return lambda: cp.start()

    def waiter(cp):
        return lambda: cp.wait()

    def dup(t):
        return jnp.concatenate([t, t], axis=0)

    def itok(src):
        if src is None:
            return jnp.uint32(16), hi_mask
        msk = (pltpu.bitcast(src, U32) | hi_mask) & hi_mask
        return dup((msk >> 12) & jnp.uint32(16)), dup(msk)

    def unpack(wd, tk):
        return pltpu.bitcast(wd << tk[0], F32), pltpu.bitcast(wd & tk[1], F32)

    def pack(a, b):
        ra = pltpu.bitcast(a.astype(BF16).astype(F32), U32)
        rb = pltpu.bitcast(b.astype(BF16).astype(F32), U32)
        return (ra >> 16) | rb

    def in_piece(xc, rg, ct, dst):
        def f(src):
            tk = itok(src)
            xs = []
            for j in range(4):
                wd = xc[pl.ds(rg * 16 * RW + ct * 4 + j, 16, stride=RW), :]
                xs.extend(unpack(wd, tk))
            v = _in_transform(xs)
            for r in range(NR):
                dst[r, ct, rg * 16:(rg + 1) * 16, :] = v[r].astype(BF16)
        return f

    def out_piece(oc, k, n, last_chunk):
        k2 = k - (CH - TAIL[-1]) // 16
        stage = last_chunk and k2 >= 0 and n in (0, 3, 4)
        saved = []

        def f0(src):
            saved.append(src)

        def f1(src):
            cols = slice(n * 128, (n + 1) * 128)
            m = [m_ref[n, r, k * 16:(k + 1) * 16, :] for r in range(NR)]
            prm = [dup(p_ref[i, :, cols]) for i in range(5)]
            if src is not None:
                tb = pltpu.bitcast(jnp.concatenate([saved[0], src], axis=0), U32)
                tok = pltpu.bitcast((tb | sign) & sign, F32)
                for r in (0, 1, 2, 3, 5, 7):
                    m[r] = m[r] + tok
            hs = _out_transform(m, *prm)
            ys = [h + h * jnp.tanh(h) for h in hs]
            for j in range(4):
                pk = pack(ys[2 * j], ys[2 * j + 1])
                if not (stage and n == NT - 1):
                    oc[pl.ds(k * 16 * RW + n * 4 + j, 16, stride=RW), :] = pk
                if stage:
                    o2_vm[pl.ds(k2 * 16 * RW + n * 4 + j, 16, stride=RW), :] = pk
        return [f0, f1]

    def u_piece(n, kb):
        def f(src):
            cols = slice(n * 128, (n + 1) * 128)
            rs = slice(kb * 32, (kb + 1) * 32)
            ks = [p_ref[i, :, cols] for i in (5, 6, 7, 8, 9, 10, 11, 2)]
            if src is not None:
                tok = pltpu.bitcast((pltpu.bitcast(src, U32) | sign) & sign, F32)
                ks = [k + tok for k in ks]
            ks = [dup(dup(k)) for k in ks]
            h0 = w_vm[n, 2, rs, :].astype(F32)
            h1 = w_vm[n, 1, rs, :].astype(F32)
            h2 = w_vm[n, 0, rs, :].astype(F32)
            for gi in range(4):
                if gi < 2:
                    k0, k1, k2 = ks[3 * gi:3 * gi + 3]
                    e = k0 * h0 + k2 * h2
                elif gi == 2:
                    k1 = ks[6]
                    e = k1 * (h0 + h2)
                else:
                    k1 = ks[7]
                    e = k1 * (h0 - h2)
                o = k1 * h1
                u_ref[n, 2 * gi, rs, :] = (e + o).astype(BF16)
                u_ref[n, 2 * gi + 1, rs, :] = (e - o).astype(BF16)
        return f

    def outs(oc, lo, M, n, last_chunk=False):
        return [f for k in range(lo // 16, (lo + M) // 16) for f in out_piece(oc, k, n, last_chunk)]

    def ins(xc, lo, M, dst):
        return [in_piece(xc, rg, ct, dst)
                for rg in range(lo // 16, (lo + M) // 16) for ct in range(NT)]

    def us(n):
        return [u_piece(n, k) for k in range(C // 32)]

    def ung(l):
        return [functools.partial(f, None) for f in l]

    def xview(b0):
        return x_vm.at[rows(b0, CH), :]

    def oview(b0):
        return o_vm.at[rows(b0, CH), :]

    def unit(v, lo, M, n, r):
        vu = v.bitcast(U32)
        lhs = jnp.concatenate([vu[r, ct, lo // 2:(lo + M) // 2, :] for ct in range(NT)], axis=1)
        ru = w_vm.bitcast(U32)[n, (2, 0, 1)[r]] if r < 3 else u_ref.bitcast(U32)[n, r - 3]
        res = jnp.dot(pltpu.bitcast(lhs, BF16), pltpu.bitcast(ru, BF16), preferred_element_type=F32)
        m_ref[n, r, lo:lo + M, :] = res
        return res

    def emit(passes, ranges, before, barriers=()):
        units = [(v, lo, M, n, r) for (v, lo, M, n) in passes for r in range(NR)]
        per = [[] for _ in units]
        for items, u0, u1 in ranges:
            tot = sum(units[k][2] for k in range(u0, u1))
            k, acc = u0, 0
            for i, it in enumerate(items):
                pos = (i + 0.5) * tot / len(items)
                while pos >= acc + units[k][2]:
                    acc += units[k][2]
                    k += 1
                per[k].append(((pos - acc) / units[k][2], it))
        bars = sorted(set([0, len(units)] + list(barriers)))
        nsplit = {}
        for b0, b1 in zip(bars[:-1], bars[1:]):
            cand = list(range(max(b0, b1 - 4), b1))
            best = None
            for combo in itertools.product((1, 2, 4), repeat=len(cand)):
                sp = dict(zip(cand, combo))
                if any(units[k][2] // v < 32 for k, v in sp.items() if v > 1):
                    continue
                load, t = [0] * 4, 0
                for k in range(b0, b1):
                    v = sp.get(k, 1)
                    for _ in range(v * NT):
                        load[t % 4] += units[k][2] // v
                        t += 1
                key = (max(load), sum(combo))
                if best is None or key < best[0]:
                    best = (key, sp)
            nsplit.update(best[1])
        for ix, (v, lo, M, n, r) in enumerate(units):
            for f in before.get(ix, ()):
                f()
            ns = nsplit.get(ix, 1)
            parts = [unit(v, lo + q * (M // ns), M // ns, n, r) for q in range(ns)]
            pm = M // len(parts)
            for fr, it in sorted(per[ix], key=lambda t: t[0]):
                rr = int(fr * (M // 8)) * 8
                it(parts[rr // pm][rr % pm:rr % pm + 8, :])
        for f in before.get(len(units), ()):
            f()

    qoff = [sum(HQ[:i]) for i in range(NQ)]
    xq = [x_copy(qoff[i], HQ[i], 1 + i) for i in range(NQ)]
    x1c = x_copy(CH, CH, s_x1)

    def xp(i):
        return x_copy((2 * i + 2) * CH, 2 * CH, s_xp + i)

    def oc_(k):
        return o_rows(rows(k * CH, CH))

    pv = [pv0, pv1, pv2, pv3]
    pcs = [pltpu.make_async_copy(r, pv[i], sem.at[0])
           for i, r in enumerate((mean_hbm, var_hbm, g_hbm, b_hbm))]
    for cp in pcs:
        cp.start()
    w_copy(0).start()
    for cp in xq:
        cp.start()
    for n in range(1, NT):
        w_copy(n).start()
    x1c.start()
    for i in range((NC - 2) // 2):
        xp(i).start()

    for cp in pcs:
        cp.wait()
    w_copy(0).wait()
    mean, var, g, b = [r[...].astype(F32).reshape(1, C) for r in pv]
    sc = 0.5 * g * jax.lax.rsqrt(var + 1e-5)
    sh = 0.5 * b - mean * sc
    prm = [sc, _KAP * sc, _KC * sc, sh, (1.0 + _KAP) * sh,
           _FA * sc, (_FA * A_PT) * sc, (_FA * _AL) * sc,
           _FB * sc, (_FB / A_PT) * sc, (_FB * _BE) * sc, _K1 * sc]
    for i, v in enumerate(prm):
        p_ref[i] = jnp.broadcast_to(v, (8, C))

    x0, o0, x1, o1 = xview(0), oview(0), xview(CH), oview(CH)
    for f in us(0):
        f(None)
    xq[0].wait()
    for f in ins(x0, 0, HQ[0], va_ref):
        f(None)
    passes = ([(va_ref, qoff[i], HQ[i], 0) for i in range(NQ)]
              + [(va_ref, 0, CH, n) for n in range(1, NT)]
              + [(vb_ref, 0, CH, 0), (vb_ref, 0, CH, 1)])
    N1 = (NQ - 1) * NR
    E, Q = HE, 1
    b2, b3, b4 = N1 + 2 * NR - HD, N1 + 3 * NR - HD, N1 + 4 * NR - HD + HX
    before = {i * NR: [waiter(xq[i + 1])] + ung(ins(x0, qoff[i + 1], HQ[i + 1], va_ref))
              for i in range(NQ - 1)}
    before[N1] = [waiter(w_copy(1))]
    before[b2] = [waiter(w_copy(2))]
    before[b3] = [waiter(w_copy(3)), waiter(w_copy(4))]
    before[b4] = [waiter(x1c)]
    barriers = list(before)
    oo0, oo1 = outs(o0, 0, CH, 0), outs(o0, 0, CH, 1)
    if NO:
        before[b2] += ung(oo0[-NO:])
        oo0 = oo0[:-NO]
    if NO1:
        before[b3] += ung(oo1[-NO1:])
        oo1 = oo1[:-NO1]
    before[N1 + 7 * NR] = [starter(oc_(0))]
    ranges = [
        (us(1), N1, N1 + NR + HE1),
        (us(2), b2, N1 + 2 * NR + E),
        (us(3), b3, N1 + 3 * NR + E),
        (us(4), N1 + 3 * NR + E, b4 - Q),
        (ins(x1, 0, CH, vb_ref), b4, N1 + 5 * NR - 1),
        (oo0, N1 + NR + E, b2 - Q),
        (oo1, N1 + 2 * NR + E, b3 - Q),
        (outs(o0, 0, CH, 2) + outs(o0, 0, CH, 3) + outs(o0, 0, CH, 4) + outs(o1, 0, CH, 0),
         N1 + 5 * NR - 1, N1 + 7 * NR - Q),
    ]
    emit(passes, ranges, before, barriers)

    def body(i, carry):
        c = 2 * i + 1
        xp(i).wait()
        oa, ob, oc = oview(c * CH), oview((c + 1) * CH), oview((c + 2) * CH)
        passes = ([(vb_ref, 0, CH, n) for n in range(2, NT)]
                  + [(va_ref, 0, CH, n) for n in range(NT)]
                  + [(vb_ref, 0, CH, 0), (vb_ref, 0, CH, 1)])
        ol = ([outs(oa, 0, CH, n) for n in range(1, NT)]
              + [outs(ob, 0, CH, n) for n in range(NT)] + [outs(oc, 0, CH, 0, True)])
        last = 2 * NT - 1
        ranges = [(ol[k], k * NR, (k + 1) * NR - (1 if k == last else 0)) for k in range(2 * NT)]
        ranges.append((ins(xview((c + 1) * CH), 0, CH, va_ref), 0, (NT - 2) * NR - 1))
        ranges.append((ins(xview((c + 2) * CH), 0, CH, vb_ref), (NT - 2) * NR, (2 * NT - 2) * NR - 1))
        before = {(NT - 1) * NR: [starter(oc_(c))], last * NR: [starter(oc_(c + 1))]}
        emit(passes, ranges, before)
        return carry

    jax.lax.fori_loop(0, (NC - 2) // 2, body, 0)

    c = NC - 1
    oc = oview(c * CH)
    passes, before = [], {}
    ranges = [(outs(oc, 0, CH, 1), 0, NR)]
    lo = 0
    for ti, M in enumerate(TAIL):
        for n in range(2, NT):
            u0 = len(passes) * NR
            passes.append((vb_ref, lo, M, n))
            if n < NT - 1:
                ranges.append((outs(oc, lo, M, n, True), u0 + NR, u0 + 2 * NR))
            elif ti < len(TAIL) - 1:
                ranges.append((outs(oc, lo, M, n), u0 + NR, u0 + NR + TQ))
                before[u0 + NR + TQ] = [starter(o_rows(rows(c * CH + lo, M)))]
        lo += M
    M = TAIL[-1]
    lo -= M
    base = (c * CH + lo) * RW
    its, u0, _ = ranges[-1]
    ranges[-1] = (its, u0, u0 + FINE)
    before[u0 + FINE] = [starter(o_rows(pl.ds(base + p * 2 * RW + r0, nr)))
                         for p in range(M // 2) for r0, nr in ((0, 16), (24, 8))]
    ol = outs(oc, lo, M, NT - 1, True)
    fl = []
    for q in range(M // 16):
        fl += ung(ol[2 * q:2 * q + 2])
        for p in range(8 * q, 8 * q + 8):
            for r0 in (16, 32):
                fl.append(starter(pltpu.make_async_copy(
                    o2_vm.at[pl.ds(p * 2 * RW + r0, 8), :],
                    oh.at[pl.ds(base + p * 2 * RW + r0, 8), :], sem.at[s_out])))
    before[len(passes) * NR] = fl
    emit(passes, ranges, before)
    pltpu.make_async_copy(oh, oh, sem.at[s_out]).wait()


@jax.jit
def pallas_standalone__batchnorm__sampling_kernel(x, w, mean, var, g, b):
    B, S, C = x.shape
    NT = C // 128
    assert S == 8 and NT == 5 and B % (2 * CH) == 0 and w.shape == (3, C, C)
    z = x.reshape(B, S, NT, 128).transpose(0, 2, 1, 3).reshape(B * S * NT, 128)
    anyspec = pl.BlockSpec(memory_space=pl.ANY)
    scratch = [
        pltpu.VMEM((B * 4 * NT, 128), U32),
        pltpu.VMEM((B * 4 * NT, 128), U32),
        pltpu.VMEM((TAIL[-1] * 4 * NT, 128), U32),
        pltpu.VMEM((NT, 3, C, 128), BF16),
        pltpu.VMEM((NT, NR - 3, C, 128), BF16),
        pltpu.VMEM((12, 8, C), F32),
        pltpu.VMEM((C,), BF16), pltpu.VMEM((C,), BF16),
        pltpu.VMEM((C,), BF16), pltpu.VMEM((C,), BF16),
        pltpu.VMEM((NR, NT, CH, 128), BF16),
        pltpu.VMEM((NR, NT, CH, 128), BF16),
        pltpu.VMEM((NT, NR, CH, 128), F32),
        pltpu.SemaphoreType.DMA((len(HQ) + 6 + (B // CH - 2) // 2,)),
    ]
    out = pl.pallas_call(
        functools.partial(_kernel, B=B, C=C),
        in_specs=[anyspec] * 6,
        out_specs=anyspec,
        out_shape=jax.ShapeDtypeStruct((B * S * NT, 128), x.dtype),
        scratch_shapes=scratch,
        compiler_params=pltpu.CompilerParams(vmem_limit_bytes=64 * 1024 * 1024),
    )(z, w, mean, var, g, b)
    return out.reshape(B, NT, S, 128).transpose(0, 2, 1, 3).reshape(B, S, C)
```

```python
import functools
import itertools

import jax
import jax.numpy as jnp
import jax.experimental.pallas as pl
import jax.experimental.pallas.tpu as pltpu

F32 = jnp.float32
BF16 = jnp.bfloat16
U32 = jnp.uint32

NR = 11
CH = 128
A_PT = 1.9
_AL = A_PT * A_PT
_BE = 1.0 / _AL
_KAP = _AL + _BE
_C1 = (A_PT + 1.0 / A_PT) / 2.0
_S1 = (A_PT - 1.0 / A_PT) / 2.0
_R = _S1 / _C1
_FA = (A_PT ** 3 * _C1) / (2.0 * _AL * (_AL * _AL - 1.0) * (_AL - _BE))
_FB = _AL * (_C1 / A_PT ** 4) / (2.0 * _BE * (_BE * _BE - 1.0) * (_BE - _AL))
_K1 = 1.0 / (4.0 * (2.0 - _KAP))
_KC = 1.0 / (2.0 * (2.0 + _KAP))

HQ = (32, 32, 32, 32)
HD = 5
HX = 4
HE = 2
HE1 = 2
NO = 8
NO1 = 8
TAIL = (64, 32, 32)
TQ = 4
FINE = 3
IG = 64
OG = 64


def _in_transform(x):
    x0, x1, x2, x3, x4, x5, x6, x7 = x

    def half(p0, p2, p4, p6):
        s06 = p0 + p6
        s24 = p2 + p4
        d60 = p6 - p0
        d42 = p4 - p2
        s = (_KAP - 1.0) * s06 + s24
        d = (_R * (_KAP + 1.0)) * d60 + _R * d42
        return s06 + s24, d42 - d60, s + d, s - d

    e1, ar, ep, em = half(x0, x2, x4, x6)
    o1, ai, op, om = half(x1, x3, x5, x7)
    em = A_PT * em
    op = A_PT * op
    return [x0, x7, ar + ai,
            ep + op, ep - op, em + om, em - om,
            e1 + o1, e1 - o1, ar, ai]


def _out_transform(m, sc, ksc, csc, sh, sh2):
    m0, mi, mk, mpa, mma, mpb, mmb, mp1, mm1, k2, k3 = m
    sa = mpa + mma
    da = mpa - mma
    sb = mpb + mmb
    db = mpb - mmb
    s1 = mp1 + mm1
    d1_ = mp1 - mm1
    k1 = csc * mk
    nre = k1 - k2
    im = k1 + k3
    e0 = sc * m0
    ke0 = ksc * m0 - sh
    d0 = s1 + nre
    d1 = s1 - nre + sh
    e2 = d1 - e0
    c1 = sa + _BE * sb
    nc0 = _BE * sa + sb
    z2 = d0 - ke0 + nc0
    z4 = d1 - _KAP * d0 - c1
    z6 = (d0 + sh2) - _KAP * e2 - nc0
    z8 = e2 + c1
    f0 = sc * mi
    kf0 = ksc * mi - sh
    g0 = d1_ + im + sh
    g1 = d1_ - im
    f2 = g0 - f0
    c1p = A_PT * da + (A_PT ** -3) * db
    nc0p = (1.0 / A_PT) * (da + db)
    z1 = f2 + nc0p
    z3 = (g1 + sh2) - _KAP * f2 - c1p
    z5 = g0 - _KAP * g1 - nc0p
    z7 = g1 - kf0 + c1p
    return [z1, z2, z3, z4, z5, z6, z7, z8]


def _kernel(x_hbm, w_hbm, mean_hbm, var_hbm, g_hbm, b_hbm, o_hbm,
            x_vm, o_vm, o2_vm, w_vm, u_ref, p_ref, pv0, pv1, pv2, pv3,
            va_ref, vb_ref, m_ref, sem, *, B, C):
    NT = C // 128
    RW = 4 * NT
    NC = B // CH
    NQ = len(HQ)
    xh = x_hbm.bitcast(U32)
    oh = o_hbm.bitcast(U32)
    hi_mask = jnp.uint32(0xFFFF0000)
    sign = jnp.uint32(0x80000000)

    s_w = {0: 0, 1: NQ + 1, 2: NQ + 2, 3: NQ + 3, 4: NQ + 3}
    s_x1 = NQ + 4
    s_xp = NQ + 5
    s_out = s_xp + (NC - 2) // 2

    def rows(b0, nb):
        if isinstance(b0, int):
            return pl.ds(b0 * RW, nb * RW)
        return pl.ds(pl.multiple_of(b0 * RW, 8), nb * RW)

    def x_copy(b0, nb, s):
        r = rows(b0, nb)
        return pltpu.make_async_copy(xh.at[r, :], x_vm.at[r, :], sem.at[s])

    def o_rows(r):
        return pltpu.make_async_copy(o_vm.at[r, :], oh.at[r, :], sem.at[s_out])

    def w_copy(n):
        return pltpu.make_async_copy(
            w_hbm.at[:, :, pl.ds(n * 128, 128)], w_vm.at[n], sem.at[s_w[n]])

    def starter(cp):
        return lambda: cp.start()

    def waiter(cp):
        return lambda: cp.wait()

    def rep(t, k):
        return jnp.concatenate([t] * k, axis=0)

    def itok(srcs):
        if srcs[0] is None:
            return jnp.uint32(16), hi_mask
        msk = (pltpu.bitcast(jnp.concatenate(srcs, axis=0), U32) | hi_mask) & hi_mask
        sft = (msk >> 12) & jnp.uint32(16)
        return tuple(jnp.concatenate([t[8 * (i // 2):8 * (i // 2) + 8] for i in range(2 * len(srcs))], axis=0)
                     for t in (sft, msk))

    def unpack(wd, tk):
        return pltpu.bitcast(wd << tk[0], F32), pltpu.bitcast(wd & tk[1], F32)

    def pack(a, b):
        ra = pltpu.bitcast(a.astype(BF16).astype(F32), U32)
        rb = pltpu.bitcast(b.astype(BF16).astype(F32), U32)
        return (ra >> 16) | (rb & hi_mask)

    def in_piece(xc, lo, ig, ct, dst):
        saved = []

        def fin(src):
            saved.append(src)
            tk = itok(saved)
            xs = []
            for j in range(4):
                xs.extend(unpack(xc[pl.ds(lo * RW + ct * 4 + j, ig, stride=RW), :], tk))
            v = _in_transform(xs)
            for r in range(NR):
                dst[r, ct, lo:lo + ig, :] = v[r].astype(BF16)
        return [saved.append] * (ig // 16 - 1) + [fin]

    def out_piece(oc, lo, og, n, last_chunk):
        lo2 = lo - (CH - TAIL[-1])
        stage = last_chunk and lo2 >= 0 and n in (0, 3, 4)
        saved = []

        def fin(src):
            saved.append(src)
            cols = slice(n * 128, (n + 1) * 128)
            m = [m_ref[n, r, lo:lo + og, :] for r in range(NR)]
            prm = [rep(p_ref[i, :, cols], og // 8) for i in range(5)]
            if src is not None:
                tb = pltpu.bitcast(jnp.concatenate(saved, axis=0), U32)
                tok = pltpu.bitcast((tb | sign) & sign, F32)
                for r in (0, 1, 2, 3, 5, 7):
                    m[r] = m[r] + tok
            hs = _out_transform(m, *prm)
            ys = [h + h * jnp.tanh(h) for h in hs]
            for j in range(4):
                pk = pack(ys[2 * j], ys[2 * j + 1])
                if not (stage and n == NT - 1):
                    oc[pl.ds(lo * RW + n * 4 + j, og, stride=RW), :] = pk
                if stage:
                    o2_vm[pl.ds(lo2 * RW + n * 4 + j, og, stride=RW), :] = pk
        return [saved.append] * (og // 8 - 1) + [fin]

    def u_piece(n, kb):
        def f(src):
            cols = slice(n * 128, (n + 1) * 128)
            rs = slice(kb * 32, (kb + 1) * 32)
            ks = [p_ref[i, :, cols] for i in (5, 6, 7, 8, 9, 10, 11, 2)]
            if src is not None:
                tok = pltpu.bitcast((pltpu.bitcast(src, U32) | sign) & sign, F32)
                ks = [k + tok for k in ks]
            ks = [rep(k, 4) for k in ks]
            h0 = w_vm[n, 2, rs, :].astype(F32)
            h1 = w_vm[n, 1, rs, :].astype(F32)
            h2 = w_vm[n, 0, rs, :].astype(F32)
            for gi in range(4):
                if gi < 2:
                    k0, k1, k2 = ks[3 * gi:3 * gi + 3]
                    e = k0 * h0 + k2 * h2
                elif gi == 2:
                    k1 = ks[6]
                    e = k1 * (h0 + h2)
                else:
                    k1 = ks[7]
                    e = k1 * (h0 - h2)
                o = k1 * h1
                u_ref[n, 2 * gi, rs, :] = (e + o).astype(BF16)
                u_ref[n, 2 * gi + 1, rs, :] = (e - o).astype(BF16)
        return f

    def outs(oc, lo, M, n, last_chunk=False, og=None):
        og = og or min(OG, M, TAIL[-1] if last_chunk else M)
        return [f for l in range(lo, lo + M, og) for f in out_piece(oc, l, og, n, last_chunk)]

    def ins(xc, lo, M, dst, ig=None):
        ig = ig or IG
        return [f for l in range(lo, lo + M, ig) for ct in range(NT)
                for f in in_piece(xc, l, ig, ct, dst)]

    def us(n):
        return [u_piece(n, k) for k in range(C // 32)]

    def ung(l):
        return [functools.partial(f, None) for f in l]

    def xview(b0):
        return x_vm.at[rows(b0, CH), :]

    def oview(b0):
        return o_vm.at[rows(b0, CH), :]

    def unit(v, lo, M, n, r):
        vu = v.bitcast(U32)
        lhs = jnp.concatenate([vu[r, ct, lo // 2:(lo + M) // 2, :] for ct in range(NT)], axis=1)
        ru = w_vm.bitcast(U32)[n, (2, 0, 1)[r]] if r < 3 else u_ref.bitcast(U32)[n, r - 3]
        res = jnp.dot(pltpu.bitcast(lhs, BF16), pltpu.bitcast(ru, BF16), preferred_element_type=F32)
        m_ref[n, r, lo:lo + M, :] = res
        return res

    def emit(passes, ranges, before, barriers=()):
        units = [(v, lo, M, n, r) for (v, lo, M, n) in passes for r in range(NR)]
        per = [[] for _ in units]
        for items, u0, u1 in ranges:
            tot = sum(units[k][2] for k in range(u0, u1))
            k, acc = u0, 0
            for i, it in enumerate(items):
                pos = (i + 0.5) * tot / len(items)
                while pos >= acc + units[k][2]:
                    acc += units[k][2]
                    k += 1
                per[k].append(((pos - acc) / units[k][2], it))
        bars = sorted(set([0, len(units)] + list(barriers)))
        nsplit = {}
        for b0, b1 in zip(bars[:-1], bars[1:]):
            cand = list(range(max(b0, b1 - 4), b1))
            best = None
            for combo in itertools.product((1, 2, 4), repeat=len(cand)):
                sp = dict(zip(cand, combo))
                if any(units[k][2] // v < 32 for k, v in sp.items() if v > 1):
                    continue
                load, t = [0] * 4, 0
                for k in range(b0, b1):
                    v = sp.get(k, 1)
                    for _ in range(v * NT):
                        load[t % 4] += units[k][2] // v
                        t += 1
                key = (max(load), sum(combo))
                if best is None or key < best[0]:
                    best = (key, sp)
            nsplit.update(best[1])
        for ix, (v, lo, M, n, r) in enumerate(units):
            for f in before.get(ix, ()):
                f()
            ns = nsplit.get(ix, 1)
            parts = [unit(v, lo + q * (M // ns), M // ns, n, r) for q in range(ns)]
            pm = M // len(parts)
            for fr, it in sorted(per[ix], key=lambda t: t[0]):
                rr = int(fr * (M // 8)) * 8
                it(parts[rr // pm][rr % pm:rr % pm + 8, :])
        for f in before.get(len(units), ()):
            f()

    qoff = [sum(HQ[:i]) for i in range(NQ)]
    xq = [x_copy(qoff[i], HQ[i], 1 + i) for i in range(NQ)]
    x1c = x_copy(CH, CH, s_x1)

    def xp(i):
        return x_copy((2 * i + 2) * CH, 2 * CH, s_xp + i)

    def oc_(k):
        return o_rows(rows(k * CH, CH))

    pv = [pv0, pv1, pv2, pv3]
    pcs = [pltpu.make_async_copy(r, pv[i], sem.at[0])
           for i, r in enumerate((mean_hbm, var_hbm, g_hbm, b_hbm))]
    for cp in pcs:
        cp.start()
    w_copy(0).start()
    for cp in xq:
        cp.start()
    for n in range(1, NT):
        w_copy(n).start()
    x1c.start()
    for i in range((NC - 2) // 2):
        xp(i).start()

    for cp in pcs:
        cp.wait()
    w_copy(0).wait()
    mean, var, g, b = [r[...].astype(F32).reshape(1, C) for r in pv]
    sc = 0.5 * g * jax.lax.rsqrt(var + 1e-5)
    sh = 0.5 * b - mean * sc
    prm = [sc, _KAP * sc, _KC * sc, sh, (1.0 + _KAP) * sh,
           _FA * sc, (_FA * A_PT) * sc, (_FA * _AL) * sc,
           _FB * sc, (_FB / A_PT) * sc, (_FB * _BE) * sc, _K1 * sc]
    for i, v in enumerate(prm):
        p_ref[i] = jnp.broadcast_to(v, (8, C))

    x0, o0, x1, o1 = xview(0), oview(0), xview(CH), oview(CH)
    for f in us(0):
        f(None)
    xq[0].wait()
    for f in ins(x0, 0, HQ[0], va_ref, 16):
        f(None)
    passes = ([(va_ref, qoff[i], HQ[i], 0) for i in range(NQ)]
              + [(va_ref, 0, CH, n) for n in range(1, NT)]
              + [(vb_ref, 0, CH, 0), (vb_ref, 0, CH, 1)])
    N1 = (NQ - 1) * NR
    E, Q = HE, 1
    b2, b3, b4 = N1 + 2 * NR - HD, N1 + 3 * NR - HD, N1 + 4 * NR - HD + HX
    before = {i * NR: [waiter(xq[i + 1])] + ung(ins(x0, qoff[i + 1], HQ[i + 1], va_ref, 16))
              for i in range(NQ - 1)}
    before[N1] = [waiter(w_copy(1))]
    before[b2] = [waiter(w_copy(2))]
    before[b3] = [waiter(w_copy(3)), waiter(w_copy(4))]
    before[b4] = [waiter(x1c)]
    barriers = list(before)
    oo0, oo1 = outs(o0, 0, CH, 0), outs(o0, 0, CH, 1)
    if NO:
        before[b2] += ung(oo0[-NO:])
        oo0 = oo0[:-NO]
    if NO1:
        before[b3] += ung(oo1[-NO1:])
        oo1 = oo1[:-NO1]
    before[N1 + 7 * NR] = [starter(oc_(0))]
    ranges = [
        (us(1), N1, N1 + NR + HE1),
        (us(2), b2, N1 + 2 * NR + E),
        (us(3), b3, N1 + 3 * NR + E),
        (us(4), N1 + 3 * NR + E, b4 - Q),
        (ins(x1, 0, CH, vb_ref), b4, N1 + 5 * NR - 1),
        (oo0, N1 + NR + E, b2 - Q),
        (oo1, N1 + 2 * NR + E, b3 - Q),
        (outs(o0, 0, CH, 2) + outs(o0, 0, CH, 3) + outs(o0, 0, CH, 4) + outs(o1, 0, CH, 0),
         N1 + 5 * NR - 1, N1 + 7 * NR - Q),
    ]
    emit(passes, ranges, before, barriers)

    def body(i, carry):
        c = 2 * i + 1
        xp(i).wait()
        oa, ob, oc = oview(c * CH), oview((c + 1) * CH), oview((c + 2) * CH)
        passes = ([(vb_ref, 0, CH, n) for n in range(2, NT)]
                  + [(va_ref, 0, CH, n) for n in range(NT)]
                  + [(vb_ref, 0, CH, 0), (vb_ref, 0, CH, 1)])
        ol = ([outs(oa, 0, CH, n) for n in range(1, NT)]
              + [outs(ob, 0, CH, n) for n in range(NT)] + [outs(oc, 0, CH, 0, True)])
        last = 2 * NT - 1
        ranges = [(ol[k], k * NR, (k + 1) * NR - (1 if k == last else 0)) for k in range(2 * NT)]
        ranges.append((ins(xview((c + 1) * CH), 0, CH, va_ref), 0, (NT - 2) * NR - 1))
        ranges.append((ins(xview((c + 2) * CH), 0, CH, vb_ref), (NT - 2) * NR, (2 * NT - 2) * NR - 1))
        before = {(NT - 1) * NR: [starter(oc_(c))], last * NR: [starter(oc_(c + 1))]}
        emit(passes, ranges, before)
        return carry

    jax.lax.fori_loop(0, (NC - 2) // 2, body, 0)

    c = NC - 1
    oc = oview(c * CH)
    passes, before = [], {}
    ranges = [(outs(oc, 0, CH, 1), 0, NR)]
    lo = 0
    for ti, M in enumerate(TAIL):
        for n in range(2, NT):
            u0 = len(passes) * NR
            passes.append((vb_ref, lo, M, n))
            if n < NT - 1:
                ranges.append((outs(oc, lo, M, n, True), u0 + NR, u0 + 2 * NR))
            elif ti < len(TAIL) - 1:
                ranges.append((outs(oc, lo, M, n), u0 + NR, u0 + NR + TQ))
                before[u0 + NR + TQ] = [starter(o_rows(rows(c * CH + lo, M)))]
        lo += M
    M = TAIL[-1]
    lo -= M
    base = (c * CH + lo) * RW
    its, u0, _ = ranges[-1]
    ranges[-1] = (its, u0, u0 + FINE)
    before[u0 + FINE] = [starter(o_rows(pl.ds(base + p * 2 * RW + r0, nr)))
                         for p in range(M // 2) for r0, nr in ((0, 16), (24, 8))]
    ol = outs(oc, lo, M, NT - 1, True, 16)
    fl = []
    for q in range(M // 16):
        fl += ung(ol[2 * q:2 * q + 2])
        for p in range(8 * q, 8 * q + 8):
            for r0 in (16, 32):
                fl.append(starter(pltpu.make_async_copy(
                    o2_vm.at[pl.ds(p * 2 * RW + r0, 8), :],
                    oh.at[pl.ds(base + p * 2 * RW + r0, 8), :], sem.at[s_out])))
    before[len(passes) * NR] = fl
    emit(passes, ranges, before)
    pltpu.make_async_copy(oh, oh, sem.at[s_out]).wait()


@jax.jit
def pallas_standalone__batchnorm__sampling_kernel(x, w, mean, var, g, b):
    B, S, C = x.shape
    NT = C // 128
    assert S == 8 and NT == 5 and B % (2 * CH) == 0 and w.shape == (3, C, C)
    z = x.reshape(B, S, NT, 128).transpose(0, 2, 1, 3).reshape(B * S * NT, 128)
    anyspec = pl.BlockSpec(memory_space=pl.ANY)
    scratch = [
        pltpu.VMEM((B * 4 * NT, 128), U32),
        pltpu.VMEM((B * 4 * NT, 128), U32),
        pltpu.VMEM((TAIL[-1] * 4 * NT, 128), U32),
        pltpu.VMEM((NT, 3, C, 128), BF16),
        pltpu.VMEM((NT, NR - 3, C, 128), BF16),
        pltpu.VMEM((12, 8, C), F32),
        pltpu.VMEM((C,), BF16), pltpu.VMEM((C,), BF16),
        pltpu.VMEM((C,), BF16), pltpu.VMEM((C,), BF16),
        pltpu.VMEM((NR, NT, CH, 128), BF16),
        pltpu.VMEM((NR, NT, CH, 128), BF16),
        pltpu.VMEM((NT, NR, CH, 128), F32),
        pltpu.SemaphoreType.DMA((len(HQ) + 6 + (B // CH - 2) // 2,)),
    ]
    out = pl.pallas_call(
        functools.partial(_kernel, B=B, C=C),
        in_specs=[anyspec] * 6,
        out_specs=anyspec,
        out_shape=jax.ShapeDtypeStruct((B * S * NT, 128), x.dtype),
        scratch_shapes=scratch,
        compiler_params=pltpu.CompilerParams(vmem_limit_bytes=64 * 1024 * 1024),
    )(z, w, mean, var, g, b)
    return out.reshape(B, NT, S, 128).transpose(0, 2, 1, 3).reshape(B, S, C)
```
